```python
import os as _os
_os.environ.setdefault("JAX_PLATFORMS", "cpu")
import jax
import jax.numpy as jnp

def _softmax(x, axis=-1):
    return jax.nn.softmax(x, axis=axis)
def _gelu(x):
    return jax.nn.gelu(x, approximate=True)
def _silu(x):
    return jax.nn.silu(x)
def _sigmoid(x):
    return jax.nn.sigmoid(x)
def _layernorm(x, axis=-1, eps=1e-5):
    m = jnp.mean(x, axis=axis, keepdims=True)
    v = jnp.var(x, axis=axis, keepdims=True)
    return (x - m) / jnp.sqrt(v + eps)
def _scatter_add(tgt, idx, src, axis=0):
    return tgt.at[idx].add(src)
def _segment_sum(src, seg, n):
    return jax.ops.segment_sum(src, seg, n)
class _Rng:
    def __init__(self, key):
        self._k = key
    def _next(self):
        self._k, sub = jax.random.split(self._k)
        return sub
    def normal(self, shape):
        return jax.random.normal(self._next(), shape, dtype=jnp.bfloat16)
    def randint(self, lo, hi, shape):
        return jax.random.randint(self._next(), shape, lo, hi, dtype=jnp.int32)
    def uniform(self, shape, lo=0.0, hi=1.0):
        return jax.random.uniform(self._next(), shape, jnp.bfloat16, lo, hi)
    def permutation(self, n):
        return jax.random.permutation(self._next(), n)


kernel_name = 'parallel_sum__mha_block__swiglu_ffn__prompt'

def setup_inputs():
    _rng = _Rng(jax.random.key(int.from_bytes(__import__("os").urandom(4), "little")))
    _w = (lambda a: (lambda t: t.astype(jnp.bfloat16) if jnp.issubdtype(t.dtype, jnp.floating) else t)(jnp.asarray(a)))
    def _A_setup():
        B, S, D, H = 1, 2048, 640, 32
        return {
            "x": _w((lambda *s: _rng.normal(s) * 0.05)(B, S, D)),
            "wqkv": _w((lambda *s: _rng.normal(s) * 0.1)(D, 3 * D)),
            "wo": _w((lambda *s: _rng.normal(s) * 0.05)(D, D)),
        }
    _A_in = _A_setup()

    def _B_setup():
        B, S, D, F = 1, 2048, 640, 1536
        return {
            "x": _w((lambda *s: _rng.normal(s) * 0.05)(B, S, D)),
            "w_gate": _w((lambda *s: _rng.normal(s) * 0.05)(D, F)),
            "w_up": _w((lambda *s: _rng.normal(s) * 0.05)(D, F)),
            "w_down": _w((lambda *s: _rng.normal(s) * 0.05)(F, D)),
        }
    _B_in = _B_setup()

    return {
        "A_x": _A_in["x"],
        "A_wqkv": _A_in["wqkv"],
        "A_wo": _A_in["wo"],
        "B_x": _B_in["x"],
        "B_w_gate": _B_in["w_gate"],
        "B_w_up": _B_in["w_up"],
        "B_w_down": _B_in["w_down"],
    }

def reference(A_x, A_wqkv, A_wo, B_x, B_w_gate, B_w_up, B_w_down):
    def _A_ref(x, wqkv, wo):
        B, S, D = x.shape
        H = 32
        Dh = D // H
        qkv = (lambda x, *d: x.transpose(*d))((x @ wqkv).reshape(B, S, 3, H, Dh), 2, 0, 3, 1, 4)
        q, k, v = qkv[0], qkv[1], qkv[2]
        scores = jnp.einsum("bhqd,bhkd->bhqk", q, k) * (Dh ** -0.5)
        p = _softmax(scores, axis=-1)
        o = jnp.einsum("bhqk,bhkd->bhqd", p, v)
        return (lambda x, *d: x.transpose(*d))(o, 0, 2, 1, 3).reshape(B, S, D) @ wo

    def _B_ref(x, w_gate, w_up, w_down):
        g = _silu(x @ w_gate)
        u = x @ w_up
        return (g * u) @ w_down

    x = A_x
    xn = _layernorm(x, axis=-1)
    return x + _A_ref(xn, A_wqkv, A_wo) + _B_ref(xn, B_w_gate, B_w_up, B_w_down)
```

```python
import math

import jax
import jax.numpy as jnp
from jax import lax
import jax.experimental.pallas as pl
import jax.experimental.pallas.tpu as pltpu

S, D, H, DH, F = 2048, 640, 32, 20, 1536
TQ = 512
TK = 128
TR = 512
NG = D // 128
NGX = 2 * NG - 1
EPS = 1e-5
QSCALE = (DH ** -0.5) * math.log2(math.e)
NT = (((1,), (1,)), ((), ()))
F32 = jnp.float32
BF16 = jnp.bfloat16


def _kernel(x_ref, wqkv_ref, wo_ref, wg_ref, wu_ref, wd_ref, o_ref,
            xn_scr, q_scr, k_scr, vt_scr, wvt_scr, s_scr, ot_scr):
    step = pl.program_id(0)

    @pl.when(step == 0)
    def _():
        wvt_scr[...] = wqkv_ref[:, 2 * D:3 * D].astype(F32).T.astype(BF16)
        lane = lax.broadcasted_iota(jnp.int32, (TR, 128), 1)
        upper = lane >= 64
        sub = lax.broadcasted_iota(jnp.int32, (32, TR), 0)

        def rows_body(r, carry):
            r0 = pl.multiple_of(r * TR, TR)
            x = x_ref[pl.ds(r0, TR), :].astype(F32)
            mu = jnp.mean(x, axis=-1, keepdims=True)
            xc = x - mu
            var = jnp.mean(xc * xc, axis=-1, keepdims=True)
            xn = (xc * lax.rsqrt(var + EPS)).astype(BF16)
            xn_scr[pl.ds(r0, TR), :] = xn
            qk = jnp.dot(xn, wqkv_ref[:, 0:2 * D], preferred_element_type=F32)
            for t, (dst, scale) in enumerate(((q_scr, QSCALE), (k_scr, None))):
                gs = []
                for g in range(NG):
                    blk = qk[:, t * D + g * 128:t * D + (g + 1) * 128]
                    if scale is not None:
                        blk = blk * scale
                    gs.append(blk)
                    dst[g, pl.ds(r0, TR), :] = blk.astype(BF16)
                for g in range(NG - 1):
                    dst[NG + g, pl.ds(r0, TR), :] = jnp.where(upper, gs[g], gs[g + 1]).astype(BF16)
            vt = lax.dot_general(wvt_scr[...], xn, NT, preferred_element_type=F32)
            for p in range(H // 2):
                ev = vt[40 * p:40 * p + 32, :]
                ev = jnp.where(sub < DH, ev, 1.0)
                if p < H // 2 - 1:
                    od = vt[40 * p + 16:40 * p + 48, :]
                else:
                    od = jnp.concatenate([vt[40 * p + 16:40 * p + 40, :], jnp.ones((8, TR), F32)], axis=0)
                od = jnp.where((sub >= 4) & (sub < 24), od, 1.0)
                vt_scr[64 * p:64 * p + 32, pl.ds(r0, TR)] = ev.astype(BF16)
                vt_scr[64 * p + 32:64 * p + 64, pl.ds(r0, TR)] = od.astype(BF16)
            return carry

        lax.fori_loop(0, S // TR, rows_body, 0)

    q0 = pl.multiple_of(step * TQ, TQ)
    nck = S // TK
    lane_q = lax.broadcasted_iota(jnp.int32, (TQ, 128), 1)

    def head_info(h):
        a = h * DH
        g = a // 128
        lo = a % 128
        gx = jnp.where(lo > 128 - DH, g + NG, g)
        return gx, lo

    def qmask(gx, lo):
        rel = (lane_q - lo) & 127
        q = q_scr[gx, pl.ds(q0, TQ), :]
        return jnp.where(rel < DH, q.astype(F32), 0.0).astype(BF16)

    def stage1_chunk(gx, qm, c, mrun):
        s = lax.dot_general(k_scr[gx, c * TK:(c + 1) * TK, :], qm, NT, preferred_element_type=F32)
        s_scr[c * TK:(c + 1) * TK, :] = s
        cm = jnp.max(s.reshape(TK // 8, 8, TQ), axis=0)
        return cm if mrun is None else jnp.maximum(mrun, cm)

    def stage2_chunk(h, m, c, acc):
        r0 = pl.multiple_of(h * 32, 32)
        p = jnp.exp2(s_scr[c * TK:(c + 1) * TK, :] - m).astype(BF16)
        o = jnp.dot(vt_scr[pl.ds(r0, 32), c * TK:(c + 1) * TK], p, preferred_element_type=F32)
        return o if acc is None else acc + o

    def fused(h_cur, m_cur, h_next):
        if h_next is not None:
            gx, lo = head_info(h_next)
            qm = qmask(gx, lo)
        mrun = None
        acc = None
        for c in range(nck):
            if h_cur is not None:
                acc = stage2_chunk(h_cur, m_cur, c, acc)
            if h_next is not None:
                mrun = stage1_chunk(gx, qm, c, mrun)
        m_next = None if h_next is None else jnp.max(mrun, axis=0, keepdims=True)
        return acc, m_next

    sub8 = lax.broadcasted_iota(jnp.int32, (8, TQ), 0)

    def finish_pair(p, acc_e, acc_o):
        inv_e = 1.0 / acc_e[24:32, :]
        inv_o = 1.0 / acc_o[24:32, :]
        r0 = pl.multiple_of(p * 40, 8)
        ot_scr[pl.ds(r0, 8), :] = acc_e[0:8, :] * inv_e
        ot_scr[pl.ds(r0 + 8, 8), :] = acc_e[8:16, :] * inv_e
        ot_scr[pl.ds(r0 + 16, 8), :] = jnp.where(sub8 < 4, acc_e[16:24, :] * inv_e, acc_o[0:8, :] * inv_o)
        ot_scr[pl.ds(r0 + 24, 8), :] = acc_o[8:16, :] * inv_o
        ot_scr[pl.ds(r0 + 32, 8), :] = acc_o[16:24, :] * inv_o

    _, m0 = fused(None, None, 0)

    def pair_body(p, m_e):
        h = 2 * p
        acc_e, m_o = fused(h, m_e, h + 1)
        acc_o, m_n = fused(h + 1, m_o, h + 2)
        finish_pair(p, acc_e, acc_o)
        return m_n

    m_e = lax.fori_loop(0, H // 2 - 1, pair_body, m0)
    acc_e, m_o = fused(H - 2, m_e, H - 1)
    acc_o, _ = fused(H - 1, m_o, None)
    finish_pair(H // 2 - 1, acc_e, acc_o)

    o = ot_scr[...].T.astype(BF16)
    attn = jnp.dot(o, wo_ref[...], preferred_element_type=F32)
    xn = xn_scr[pl.ds(q0, TQ), :]
    g = jnp.dot(xn, wg_ref[...], preferred_element_type=F32)
    u = jnp.dot(xn, wu_ref[...], preferred_element_type=F32)
    hmid = (g * jax.nn.sigmoid(g) * u).astype(BF16)
    ffn = jnp.dot(hmid, wd_ref[...], preferred_element_type=F32)
    x = x_ref[pl.ds(q0, TQ), :].astype(F32)
    o_ref[...] = (x + attn + ffn).astype(o_ref.dtype)


@jax.jit
def pallas_parallel_sum__mha_block__swiglu_ffn__prompt_kernel(
    A_x: jax.Array,
    A_wqkv: jax.Array,
    A_wo: jax.Array,
    B_x: jax.Array,
    B_w_gate: jax.Array,
    B_w_up: jax.Array,
    B_w_down: jax.Array,
):
    del B_x
    x = A_x.reshape(S, D)
    full = lambda shape: pl.BlockSpec(shape, lambda i: (0,) * len(shape))
    out = pl.pallas_call(
        _kernel,
        grid=(S // TQ,),
        in_specs=[full((S, D)), full((D, 3 * D)), full((D, D)), full((D, F)), full((D, F)), full((F, D))],
        out_specs=pl.BlockSpec((TQ, D), lambda i: (i, 0)),
        out_shape=jax.ShapeDtypeStruct((S, D), A_x.dtype),
        scratch_shapes=[
            pltpu.VMEM((S, D), BF16),
            pltpu.VMEM((NGX, S, 128), BF16),
            pltpu.VMEM((NGX, S, 128), BF16),
            pltpu.VMEM((H * 32, S), BF16),
            pltpu.VMEM((D, D), BF16),
            pltpu.VMEM((S, TQ), F32),
            pltpu.VMEM((D, TQ), F32),
        ],
        compiler_params=pltpu.CompilerParams(
            dimension_semantics=("arbitrary",),
            vmem_limit_bytes=100 * 1024 * 1024,
        ),
    )(x, A_wqkv, A_wo, B_w_gate, B_w_up, B_w_down)
    return out.reshape(1, S, D)
```

```python
import math

import jax
import jax.numpy as jnp
from jax import lax
import jax.experimental.pallas as pl
import jax.experimental.pallas.tpu as pltpu

S, D, H, DH, F = 2048, 640, 32, 20, 1536
TQ = 512
TK = 128
TR = 512

HPI = 8
LEAD = 2
NG = D // 128
NGX = 2 * NG - 1
NQ = S // TQ
NR = S // TR
EPS = 1e-5
QSCALE = (DH ** -0.5) * math.log2(math.e)
NT = (((1,), (1,)), ((), ()))
F32 = jnp.float32
BF16 = jnp.bfloat16


def _kernel(x_hbm, wqkv_hbm, wo_hbm, wg_hbm, wu_hbm, wd_hbm, o_ref,
            x_ref, wqkv_ref, wo_ref, wg_ref, wu_ref, wd_ref, sems,
            xn_scr, q_scr, k_scr, vt_scr, s2_scr, ot_scr, m_scr):
    step = pl.program_id(0)
    sa_scr = s2_scr.at[0]
    sb_scr = s2_scr.at[1]
    nck = S // TK
    lane_q = lax.broadcasted_iota(jnp.int32, (TQ, 128), 1)

    def head_info(h):
        a = h * DH
        g = a // 128
        lo = a % 128
        gx = jnp.where(lo > 128 - DH, g + NG, g)
        return gx, lo

    def qmask(gx, lo, q0):
        rel = (lane_q - lo) & 127
        q = q_scr[gx, pl.ds(q0, TQ), :]
        return jnp.where(rel < DH, q.astype(F32), 0.0).astype(BF16)

    def stage1_chunk(s_scr, gx, qm, c, mrun):
        s = lax.dot_general(k_scr[gx, c * TK:(c + 1) * TK, :], qm, NT, preferred_element_type=F32)
        s_scr[c * TK:(c + 1) * TK, :] = s
        cm = jnp.max(s.reshape(TK // 8, 8, TQ), axis=0)
        return cm if mrun is None else jnp.maximum(mrun, cm)

    def stage2_chunk(s_scr, h, m, c, acc):
        r0 = pl.multiple_of(h * 24, 8)
        p = jnp.exp2(s_scr[c * TK:(c + 1) * TK, :] - m).astype(BF16)
        o = jnp.dot(vt_scr[pl.ds(r0, 24), c * TK:(c + 1) * TK], p, preferred_element_type=F32)
        return o if acc is None else acc + o

    def s_buf(item):
        return s2_scr.at[item % 2]

    def item_q(h, qsel):
        gx, lo = head_info(h)
        return gx, qmask(gx, lo, qsel)

    def x_copy(r):
        return pltpu.make_async_copy(x_hbm.at[pl.ds(pl.multiple_of(r * TR, TR), TR), :], x_ref.at[pl.ds(pl.multiple_of(r * TR, TR), TR), :], sems.at[r])

    def w_copy(t):
        return pltpu.make_async_copy(wqkv_hbm.at[:, pl.ds(t * D, D)], wqkv_ref.at[:, pl.ds(t * D, D)], sems.at[NR + t])

    late = ((wg_hbm, wg_ref), (wu_hbm, wu_ref), (wd_hbm, wd_ref), (wo_hbm, wo_ref))

    def late_copy(t):
        return pltpu.make_async_copy(late[t][0], late[t][1], sems.at[NR + 3 + t])

    @pl.when(step == 0)
    def _():
        x_copy(0).start()
        for t in (2, 0, 1):
            w_copy(t).start()

        lane = lax.broadcasted_iota(jnp.int32, (TR, 128), 1)
        upper = lane >= 64
        low4 = lax.broadcasted_iota(jnp.int32, (8, TR), 0) < 4

        def layernorm(r0):
            x = x_ref[pl.ds(r0, TR), :].astype(F32)
            mu = jnp.mean(x, axis=-1, keepdims=True)
            xc = x - mu
            var = jnp.mean(xc * xc, axis=-1, keepdims=True)
            xn_scr[pl.ds(r0, TR), :] = (xc * lax.rsqrt(var + EPS)).astype(BF16)

        x_copy(0).wait()
        for r in range(1, NR):
            x_copy(r).start()
        layernorm(0)
        for t in range(3):
            w_copy(t).wait()
        for t in range(4):
            late_copy(t).start()

        def rows_body(r, carry):
            @pl.when(r + 1 < NR)
            def _():
                x_copy(r + 1).wait()
            r0 = pl.multiple_of(r * TR, TR)
            xn = xn_scr[pl.ds(r0, TR), :]
            vt = jnp.dot(xn, wqkv_ref[:, 2 * D:3 * D], preferred_element_type=F32).T
            for p in range(H // 2):
                mid = vt[40 * p + 16:40 * p + 24, :]
                vt_scr[48 * p:48 * p + 16, pl.ds(r0, TR)] = vt[40 * p:40 * p + 16, :]
                vt_scr[48 * p + 16:48 * p + 24, pl.ds(r0, TR)] = jnp.where(low4, mid, 1.0)
                vt_scr[48 * p + 24:48 * p + 32, pl.ds(r0, TR)] = jnp.where(low4, 1.0, mid)
                vt_scr[48 * p + 32:48 * p + 48, pl.ds(r0, TR)] = vt[40 * p + 24:40 * p + 40, :]
            qk = jnp.dot(xn, wqkv_ref[:, 0:2 * D], preferred_element_type=F32)
            for t, (dst, scale) in enumerate(((q_scr, QSCALE), (k_scr, None))):
                gs = []
                for g in range(NG):
                    blk = qk[:, t * D + g * 128:t * D + (g + 1) * 128]
                    if scale is not None:
                        blk = blk * scale
                    gs.append(blk)
                    dst[g, pl.ds(r0, TR), :] = blk.astype(BF16)
                for g in range(NG - 1):
                    dst[NG + g, pl.ds(r0, TR), :] = jnp.where(upper, gs[g], gs[g + 1]).astype(BF16)
            rn = jnp.where(r + 1 < NR, r + 1, 0)
            layernorm(pl.multiple_of(rn * TR, TR))
            return carry

        lax.fori_loop(0, NR, rows_body, 0)
        mrun = None
        gx, qm = item_q(0, 0)
        for c in range(nck):
            mrun = stage1_chunk(s_buf(0), gx, qm, c, mrun)
        m_scr[0:8, :] = jnp.broadcast_to(jnp.max(mrun, axis=0, keepdims=True), (8, TQ))
        mrun = jnp.full((8, TQ), -jnp.inf, F32)
        gx, qm = item_q(1, 0)
        for c in range(LEAD):
            mrun = stage1_chunk(s_buf(1), gx, qm, c, mrun)
        m_scr[8:16, :] = mrun
        for t in range(4):
            late_copy(t).wait()

    q0 = pl.multiple_of(step * TQ, TQ)
    q1 = pl.multiple_of(jnp.minimum(step + 1, NQ - 1) * TQ, TQ)
    low4q = lax.broadcasted_iota(jnp.int32, (8, TQ), 0) < 4

    def finish_pair(p, acc_e, acc_o):
        inv_e = 1.0 / acc_e[20:21, :]
        inv_o = 1.0 / acc_o[0:1, :]
        r0 = pl.multiple_of(p * 40, 8)
        ot_scr[pl.ds(r0, 16), :] = acc_e[0:16, :] * inv_e
        ot_scr[pl.ds(r0 + 16, 8), :] = jnp.where(low4q, acc_e[16:24, :] * inv_e, acc_o[0:8, :] * inv_o)
        ot_scr[pl.ds(r0 + 24, 16), :] = acc_o[8:24, :] * inv_o

    def body(it, carry):
        m, mrun = carry
        h0 = it * HPI
        wrap = h0 + HPI >= H
        qn = pl.multiple_of(jnp.where(wrap, q1, q0), TQ)
        hn = jnp.where(wrap, 0, h0 + HPI)
        m_next = None
        accs = []
        acc = None
        cur1 = None
        for t in range(HPI * nck):
            u = t + nck + LEAD
            i1, c1 = divmod(u, nck)
            if cur1 is None or c1 == 0:
                cur1 = item_q(h0 + i1, q0) if i1 < HPI else item_q(hn + (i1 - HPI), qn)
                if c1 == 0:
                    mrun = None
            mrun = stage1_chunk(s_buf(i1), cur1[0], cur1[1], c1, mrun)
            if c1 == nck - 1:
                m_next = jnp.max(mrun, axis=0, keepdims=True)
            i2, c2 = divmod(t, nck)
            acc = stage2_chunk(s_buf(i2), h0 + i2, m, c2, None if c2 == 0 else acc)
            if c2 == nck - 1:
                accs.append(acc)
                m = m_next
                if i2 % 2 == 1:
                    finish_pair((h0 + i2) // 2, accs[-2], accs[-1])
        if LEAD == 0:
            mrun = jnp.full((8, TQ), -jnp.inf, F32)
        return m, mrun

    m_fin, mrun_fin = lax.fori_loop(0, H // HPI, body, (m_scr[0:1, :], m_scr[8:16, :]))
    m_scr[0:8, :] = jnp.broadcast_to(m_fin, (8, TQ))
    m_scr[8:16, :] = mrun_fin

    o = ot_scr[...].T.astype(BF16)
    attn = jnp.dot(o, wo_ref[...], preferred_element_type=F32)
    xn = xn_scr[pl.ds(q0, TQ), :]
    g = jnp.dot(xn, wg_ref[...], preferred_element_type=F32)
    u = jnp.dot(xn, wu_ref[...], preferred_element_type=F32)
    hmid = (g * jax.nn.sigmoid(g) * u).astype(BF16)
    ffn = jnp.dot(hmid, wd_ref[...], preferred_element_type=F32)
    x = x_ref[pl.ds(q0, TQ), :].astype(F32)
    o_ref[...] = (x + attn + ffn).astype(o_ref.dtype)


@jax.jit
def pallas_parallel_sum__mha_block__swiglu_ffn__prompt_kernel(
    A_x: jax.Array,
    A_wqkv: jax.Array,
    A_wo: jax.Array,
    B_x: jax.Array,
    B_w_gate: jax.Array,
    B_w_up: jax.Array,
    B_w_down: jax.Array,
):
    del B_x
    x = A_x.reshape(S, D)
    hbm = pl.BlockSpec(memory_space=pl.ANY)
    out = pl.pallas_call(
        _kernel,
        grid=(NQ,),
        in_specs=[hbm] * 6,
        out_specs=pl.BlockSpec((TQ, D), lambda i: (i, 0)),
        out_shape=jax.ShapeDtypeStruct((S, D), A_x.dtype),
        scratch_shapes=[
            pltpu.VMEM((S, D), BF16),
            pltpu.VMEM((D, 3 * D), BF16),
            pltpu.VMEM((D, D), BF16),
            pltpu.VMEM((D, F), BF16),
            pltpu.VMEM((D, F), BF16),
            pltpu.VMEM((F, D), BF16),
            pltpu.SemaphoreType.DMA((NR + 7,)),
            pltpu.VMEM((S, D), BF16),
            pltpu.VMEM((NGX, S, 128), BF16),
            pltpu.VMEM((NGX, S, 128), BF16),
            pltpu.VMEM((H * 24, S), F32),
            pltpu.VMEM((2, S, TQ), F32),
            pltpu.VMEM((D, TQ), F32),
            pltpu.VMEM((16, TQ), F32),
        ],
        compiler_params=pltpu.CompilerParams(
            dimension_semantics=("arbitrary",),
            vmem_limit_bytes=100 * 1024 * 1024,
        ),
    )(x, A_wqkv, A_wo, B_w_gate, B_w_up, B_w_down)
    return out.reshape(1, S, D)
```

```python
import math

import jax
import jax.numpy as jnp
from jax import lax
import jax.experimental.pallas as pl
import jax.experimental.pallas.tpu as pltpu

S, D, H, DH, F = 2048, 640, 32, 20, 1536
TQ = 512
TK = 128
TR = 256
TO = 128
HPI = 16
LEAD = 2
FSUB = 384
NG = D // 128
NGX = 2 * NG - 1
NQ = S // TQ
NR = S // TR
NCK = S // TK
EPS = 1e-5
QSCALE = (DH ** -0.5) * math.log2(math.e)
NT = (((1,), (1,)), ((), ()))
F32 = jnp.float32
BF16 = jnp.bfloat16


def _kernel(x_hbm, wqkv_hbm, wo_hbm, wg_hbm, wu_hbm, wd_hbm, o_hbm,
            x_ref, wqkv_ref, wo_ref, wg_ref, wu_ref, wd_ref, sems,
            xn_scr, q_scr, k_scr, vt_scr, s2_scr, ot_scr, m_scr, y_scr, o_scr, osems):
    step = pl.program_id(0)
    lane_q = lax.broadcasted_iota(jnp.int32, (TQ, 128), 1)

    def item_q(h, qrow):
        a = h * DH
        g = a // 128
        lo = a % 128
        gx = jnp.where(lo > 128 - DH, g + NG, g)
        rel = (lane_q - lo) & 127
        q = q_scr[gx, pl.ds(qrow, TQ), :]
        return gx, jnp.where(rel < DH, q.astype(F32), 0.0).astype(BF16)

    def stage1_chunk(item, gx, qm, c, mrun):
        s = lax.dot_general(k_scr[gx, c * TK:(c + 1) * TK, :], qm, NT, preferred_element_type=F32)
        s2_scr[item % 2, c * TK:(c + 1) * TK, :] = s
        cm = jnp.max(s.reshape(TK // 8, 8, TQ), axis=0)
        return cm if mrun is None else jnp.maximum(mrun, cm)

    def stage2_chunk(item, h, m, c, acc):
        r0 = pl.multiple_of(h * 24, 8)
        p = jnp.exp2(s2_scr[item % 2, c * TK:(c + 1) * TK, :] - m).astype(BF16)
        return acc + jnp.dot(vt_scr[pl.ds(r0, 24), c * TK:(c + 1) * TK], p, preferred_element_type=F32)

    def x_copy(r):
        rows = pl.ds(pl.multiple_of(r * TR, TR), TR)
        return pltpu.make_async_copy(x_hbm.at[rows, :], x_ref.at[rows, :], sems.at[r])

    def w_copy(t):
        cols = pl.ds(t * D, D)
        return pltpu.make_async_copy(wqkv_hbm.at[:, cols], wqkv_ref.at[:, cols], sems.at[NR + t])

    late = ((wg_hbm, wg_ref), (wu_hbm, wu_ref), (wd_hbm, wd_ref), (wo_hbm, wo_ref))

    def late_copy(t):
        return pltpu.make_async_copy(late[t][0], late[t][1], sems.at[NR + 3 + t])

    def o_copy(j, row0):
        dst = pl.ds(pl.multiple_of(row0 + j * TO, TO), TO)
        return pltpu.make_async_copy(o_scr.at[pl.ds(j * TO, TO), :], o_hbm.at[dst, :], osems.at[j])

    @pl.when(step == 0)
    def _():
        x_copy(0).start()
        w_copy(0).start()

        upper = lax.broadcasted_iota(jnp.int32, (TR, 128), 1) >= 64
        low4 = lax.broadcasted_iota(jnp.int32, (8, TR), 0) < 4

        def layernorm(r0):
            x = x_ref[pl.ds(r0, TR), :].astype(F32)
            mu = jnp.mean(x, axis=-1, keepdims=True)
            xc = x - mu
            var = jnp.mean(xc * xc, axis=-1, keepdims=True)
            xn_scr[pl.ds(r0, TR), :] = (xc * lax.rsqrt(var + EPS)).astype(BF16)

        def v_part(xn, r0):
            vt = jnp.dot(xn, wqkv_ref[:, 2 * D:3 * D], preferred_element_type=F32).T
            for p in range(H // 2):
                mid = vt[40 * p + 16:40 * p + 24, :]
                vt_scr[48 * p:48 * p + 16, pl.ds(r0, TR)] = vt[40 * p:40 * p + 16, :]
                vt_scr[48 * p + 16:48 * p + 24, pl.ds(r0, TR)] = jnp.where(low4, mid, 1.0)
                vt_scr[48 * p + 24:48 * p + 32, pl.ds(r0, TR)] = jnp.where(low4, 1.0, mid)
                vt_scr[48 * p + 32:48 * p + 48, pl.ds(r0, TR)] = vt[40 * p + 24:40 * p + 40, :]

        def qk_part(xn, r0, t0, t1):
            qk = jnp.dot(xn, wqkv_ref[:, t0 * D:t1 * D], preferred_element_type=F32)
            for t in range(t0, t1):
                dst, scale = ((q_scr, QSCALE), (k_scr, None))[t]
                gs = []
                for g in range(NG):
                    blk = qk[:, (t - t0) * D + g * 128:(t - t0) * D + (g + 1) * 128]
                    if scale is not None:
                        blk = blk * scale
                    gs.append(blk)
                    dst[g, pl.ds(r0, TR), :] = blk.astype(BF16)
                for g in range(NG - 1):
                    dst[NG + g, pl.ds(r0, TR), :] = jnp.where(upper, gs[g], gs[g + 1]).astype(BF16)

        x_copy(0).wait()
        w_copy(2).start()
        x_copy(1).start()
        w_copy(1).start()
        layernorm(0)
        w_copy(0).wait()
        qk_part(xn_scr[0:TR, :], 0, 0, 1)
        w_copy(2).wait()
        x_copy(1).wait()
        for r in range(2, NR):
            x_copy(r).start()
        layernorm(TR)
        v_part(xn_scr[0:TR, :], 0)
        w_copy(1).wait()
        for t in range(4):
            late_copy(t).start()
        qk_part(xn_scr[0:TR, :], 0, 1, 2)

        def rows_body(r, carry):
            @pl.when(r + 1 < NR)
            def _():
                x_copy(r + 1).wait()
            r0 = pl.multiple_of(r * TR, TR)
            xn = xn_scr[pl.ds(r0, TR), :]
            v_part(xn, r0)
            qk_part(xn, r0, 0, 2)
            rn = jnp.where(r + 1 < NR, r + 1, 0)
            layernorm(pl.multiple_of(rn * TR, TR))
            return carry

        lax.fori_loop(1, NR, rows_body, 0)

        mrun = None
        gx, qm = item_q(0, 0)
        for c in range(NCK):
            mrun = stage1_chunk(0, gx, qm, c, mrun)
        m_scr[0:8, :] = jnp.broadcast_to(jnp.max(mrun, axis=0, keepdims=True), (8, TQ))
        mrun = None
        gx, qm = item_q(1, 0)
        for c in range(LEAD):
            mrun = stage1_chunk(1, gx, qm, c, mrun)
        m_scr[8:16, :] = mrun
        m_scr[16:40, :] = jnp.zeros((24, TQ), F32)
        y_scr[...] = jnp.zeros((TQ, D), F32)
        for t in range(4):
            late_copy(t).wait()

    q0 = pl.multiple_of(step * TQ, TQ)
    q1 = pl.multiple_of(jnp.minimum(step + 1, NQ - 1) * TQ, TQ)
    low4q = lax.broadcasted_iota(jnp.int32, (8, TQ), 0) < 4

    def finish_pair(p, acc_e, acc_o):
        inv_e = 1.0 / acc_e[20:21, :]
        inv_o = 1.0 / acc_o[0:1, :]
        r0 = pl.multiple_of(p * 40, 8)
        ot_scr[pl.ds(r0, 16), :] = acc_e[0:16, :] * inv_e
        ot_scr[pl.ds(r0 + 16, 8), :] = jnp.where(low4q, acc_e[16:24, :] * inv_e, acc_o[0:8, :] * inv_o)
        ot_scr[pl.ds(r0 + 24, 16), :] = acc_o[8:24, :] * inv_o

    def body(it, carry):
        m, mrun = carry
        h0 = it * HPI
        wrap = h0 + HPI >= H
        qn = pl.multiple_of(jnp.where(wrap, q1, q0), TQ)
        hn = jnp.where(wrap, 0, h0 + HPI)
        fc = F // (H // HPI)
        nsub = fc // FSUB
        hidden = {}

        def ffn_up(j):
            c0 = pl.multiple_of(it * fc + j * FSUB, 128)
            xn = xn_scr[pl.ds(q0, TQ), :]
            g = jnp.dot(xn, wg_ref[:, pl.ds(c0, FSUB)], preferred_element_type=F32)
            u = jnp.dot(xn, wu_ref[:, pl.ds(c0, FSUB)], preferred_element_type=F32)
            hidden[j] = (g * jax.nn.sigmoid(g) * u).astype(BF16)

        def ffn_down(j):
            c0 = pl.multiple_of(it * fc + j * FSUB, 128)
            part = jnp.dot(hidden.pop(j), wd_ref[pl.ds(c0, FSUB), :], preferred_element_type=F32)
            if j == 0:
                prev = jnp.where(it == 0, x_ref[pl.ds(q0, TQ), :].astype(F32), y_scr[...])
            else:
                prev = y_scr[...]
            y_scr[...] = prev + part

        total = HPI * NCK
        ffn_at = {}
        for j in range(nsub):
            ffn_at[(2 * j) * total // (2 * nsub)] = (ffn_up, j)
            ffn_at[(2 * j + 1) * total // (2 * nsub)] = (ffn_down, j)

        m_next = None
        accs = []
        acc = None
        cur = None
        for t in range(total):
            if t in ffn_at:
                ffn_at[t][0](ffn_at[t][1])
            i1, c1 = divmod(t + NCK + LEAD, NCK)
            if cur is None or c1 == 0:
                cur = item_q(h0 + i1, q0) if i1 < HPI else item_q(hn + (i1 - HPI), qn)
                if c1 == 0:
                    mrun = None
            mrun = stage1_chunk(i1, cur[0], cur[1], c1, mrun)
            if c1 == NCK - 1:
                m_next = jnp.max(mrun, axis=0, keepdims=True)
            i2, c2 = divmod(t, NCK)
            acc = stage2_chunk(i2, h0 + i2, m, c2, m_scr[16:40, :] if c2 == 0 else acc)
            if c2 == NCK - 1:
                accs.append(acc)
                m = m_next
                if i2 % 2 == 1:
                    finish_pair((h0 + i2) // 2, accs[-2], accs[-1])
        return m, mrun

    m_fin, mrun_fin = lax.fori_loop(0, H // HPI, body, (m_scr[0:1, :], m_scr[8:16, :]))
    m_scr[0:8, :] = jnp.broadcast_to(m_fin, (8, TQ))
    m_scr[8:16, :] = mrun_fin

    @pl.when(step > 0)
    def _():
        for j in range(TQ // TO):
            o_copy(j, q0 - TQ).wait()

    for j in range(TQ // TO):
        o = ot_scr[:, j * TO:(j + 1) * TO].T.astype(BF16)
        attn = jnp.dot(o, wo_ref[...], preferred_element_type=F32)
        o_scr[j * TO:(j + 1) * TO, :] = (y_scr[j * TO:(j + 1) * TO, :] + attn).astype(BF16)
        o_copy(j, q0).start()

    @pl.when(step == NQ - 1)
    def _():
        for j in range(TQ // TO):
            o_copy(j, q0).wait()


@jax.jit
def pallas_parallel_sum__mha_block__swiglu_ffn__prompt_kernel(
    A_x: jax.Array,
    A_wqkv: jax.Array,
    A_wo: jax.Array,
    B_x: jax.Array,
    B_w_gate: jax.Array,
    B_w_up: jax.Array,
    B_w_down: jax.Array,
):
    del B_x
    x = A_x.reshape(S, D)
    hbm = pl.BlockSpec(memory_space=pl.ANY)
    out = pl.pallas_call(
        _kernel,
        grid=(NQ,),
        in_specs=[hbm] * 6,
        out_specs=hbm,
        out_shape=jax.ShapeDtypeStruct((S, D), A_x.dtype),
        scratch_shapes=[
            pltpu.VMEM((S, D), BF16),
            pltpu.VMEM((D, 3 * D), BF16),
            pltpu.VMEM((D, D), BF16),
            pltpu.VMEM((D, F), BF16),
            pltpu.VMEM((D, F), BF16),
            pltpu.VMEM((F, D), BF16),
            pltpu.SemaphoreType.DMA((NR + 7,)),
            pltpu.VMEM((S, D), BF16),
            pltpu.VMEM((NGX, S, 128), BF16),
            pltpu.VMEM((NGX, S, 128), BF16),
            pltpu.VMEM((H * 24, S), F32),
            pltpu.VMEM((2, S, TQ), F32),
            pltpu.VMEM((D, TQ), F32),
            pltpu.VMEM((40, TQ), F32),
            pltpu.VMEM((TQ, D), F32),
            pltpu.VMEM((TQ, D), BF16),
            pltpu.SemaphoreType.DMA((TQ // TO,)),
        ],
        compiler_params=pltpu.CompilerParams(
            dimension_semantics=("arbitrary",),
            vmem_limit_bytes=100 * 1024 * 1024,
        ),
    )(x, A_wqkv, A_wo, B_w_gate, B_w_up, B_w_down)
    return out.reshape(1, S, D)
```

```python
import math

import jax
import jax.numpy as jnp
from jax import lax
import jax.experimental.pallas as pl
import jax.experimental.pallas.tpu as pltpu

S, D, H, DH, F = 2048, 640, 32, 20, 1536
TQ = 512
TK = 128
TR = 256
TO = 128
HPI = 16
NSP = 4
LEAD = 2
FSUB = 768
NG = D // 128
NGX = 2 * NG - 1
NQ = S // TQ
NR = S // TR
NCK = S // TK
NCS = NCK // NSP
EPS = 1e-5
QSCALE = (DH ** -0.5) * math.log2(math.e)
NT = (((1,), (1,)), ((), ()))
F32 = jnp.float32
BF16 = jnp.bfloat16


def _kernel(x_hbm, wqkv_hbm, wo_hbm, wg_hbm, wu_hbm, wd_hbm, o_hbm,
            x_ref, wqkv_ref, wo_ref, wg_ref, wu_ref, wd_ref, sems,
            xn_scr, q_scr, k_scr, vt_scr, s2_scr, ot_scr, m_scr, y_scr, o_scr, osems):
    step = pl.program_id(0)
    lane_q = lax.broadcasted_iota(jnp.int32, (TQ, 128), 1)

    def item_q(h, qrow):
        a = h * DH
        g = a // 128
        lo = a % 128
        gx = jnp.where(lo > 128 - DH, g + NG, g)
        rel = (lane_q - lo) & 127
        q = q_scr[gx, pl.ds(qrow, TQ), :]
        return gx, jnp.where(rel < DH, q.astype(F32), 0.0).astype(BF16)

    def stage1_chunk(item, gx, qm, c, mrun):
        s = lax.dot_general(k_scr[gx, c * TK:(c + 1) * TK, :], qm, NT, preferred_element_type=F32)
        cs = c % NCS
        s2_scr[item % 2, cs * TK:(cs + 1) * TK, :] = s
        cm = jnp.max(s.reshape(TK // 8, 8, TQ), axis=0)
        return cm if mrun is None else jnp.maximum(mrun, cm)

    def stage2_chunk(item, h, m, c, acc):
        r0 = pl.multiple_of(h * 24, 8)
        cs = c % NCS
        p = jnp.exp2(s2_scr[item % 2, cs * TK:(cs + 1) * TK, :] - m).astype(BF16)
        return acc + jnp.dot(vt_scr[pl.ds(r0, 24), c * TK:(c + 1) * TK], p, preferred_element_type=F32)

    def x_copy(r):
        rows = pl.ds(pl.multiple_of(r * TR, TR), TR)
        return pltpu.make_async_copy(x_hbm.at[rows, :], x_ref.at[rows, :], sems.at[r])

    def w_copy(t):
        cols = pl.ds(t * D, D)
        return pltpu.make_async_copy(wqkv_hbm.at[:, cols], wqkv_ref.at[:, cols], sems.at[NR + t])

    late = ((wg_hbm, wg_ref), (wu_hbm, wu_ref), (wd_hbm, wd_ref), (wo_hbm, wo_ref))

    def late_copy(t):
        return pltpu.make_async_copy(late[t][0], late[t][1], sems.at[NR + 3 + t])

    def o_copy(j, row0):
        dst = pl.ds(pl.multiple_of(row0 + j * TO, TO), TO)
        return pltpu.make_async_copy(o_scr.at[pl.ds(j * TO, TO), :], o_hbm.at[dst, :], osems.at[j])

    @pl.when(step == 0)
    def _():
        x_copy(0).start()
        w_copy(0).start()
        m_scr[16:40, :] = jnp.zeros((24, TQ), F32)
        y_scr[...] = jnp.zeros((TQ, D), F32)

        upper = lax.broadcasted_iota(jnp.int32, (TR, 128), 1) >= 64
        low4 = lax.broadcasted_iota(jnp.int32, (8, TR), 0) < 4

        def layernorm(r0):
            x = x_ref[pl.ds(r0, TR), :].astype(F32)
            mu = jnp.mean(x, axis=-1, keepdims=True)
            xc = x - mu
            var = jnp.mean(xc * xc, axis=-1, keepdims=True)
            xn_scr[pl.ds(r0, TR), :] = (xc * lax.rsqrt(var + EPS)).astype(BF16)

        def v_part(xn, r0):
            vt = jnp.dot(xn, wqkv_ref[:, 2 * D:3 * D], preferred_element_type=F32).T
            for p in range(H // 2):
                mid = vt[40 * p + 16:40 * p + 24, :]
                vt_scr[48 * p:48 * p + 16, pl.ds(r0, TR)] = vt[40 * p:40 * p + 16, :]
                vt_scr[48 * p + 16:48 * p + 24, pl.ds(r0, TR)] = jnp.where(low4, mid, 1.0)
                vt_scr[48 * p + 24:48 * p + 32, pl.ds(r0, TR)] = jnp.where(low4, 1.0, mid)
                vt_scr[48 * p + 32:48 * p + 48, pl.ds(r0, TR)] = vt[40 * p + 24:40 * p + 40, :]

        def qk_part(xn, r0, t0, t1):
            qk = jnp.dot(xn, wqkv_ref[:, t0 * D:t1 * D], preferred_element_type=F32)
            for t in range(t0, t1):
                dst, scale = ((q_scr, QSCALE), (k_scr, None))[t]
                gs = []
                for g in range(NG):
                    blk = qk[:, (t - t0) * D + g * 128:(t - t0) * D + (g + 1) * 128]
                    if scale is not None:
                        blk = blk * scale
                    gs.append(blk)
                    dst[g, pl.ds(r0, TR), :] = blk.astype(BF16)
                for g in range(NG - 1):
                    dst[NG + g, pl.ds(r0, TR), :] = jnp.where(upper, gs[g], gs[g + 1]).astype(BF16)

        x_copy(0).wait()
        w_copy(2).start()
        x_copy(1).start()
        w_copy(1).start()
        layernorm(0)
        w_copy(0).wait()
        qk_part(xn_scr[0:TR, :], 0, 0, 1)
        w_copy(2).wait()
        x_copy(1).wait()
        for r in range(2, NR):
            x_copy(r).start()
        layernorm(TR)
        v_part(xn_scr[0:TR, :], 0)
        w_copy(1).wait()
        for t in range(4):
            late_copy(t).start()
        qk_part(xn_scr[0:TR, :], 0, 1, 2)

        def rows_body(r, carry):
            @pl.when(r + 1 < NR)
            def _():
                x_copy(r + 1).wait()
            r0 = pl.multiple_of(r * TR, TR)
            xn = xn_scr[pl.ds(r0, TR), :]
            v_part(xn, r0)
            qk_part(xn, r0, 0, 2)
            rn = jnp.where(r + 1 < NR, r + 1, 0)
            layernorm(pl.multiple_of(rn * TR, TR))
            return carry

        lax.fori_loop(1, NR, rows_body, 0)

        cur = None
        mrun = None
        for u in range(NCS + LEAD):
            i1, c1 = divmod(u, NCK)
            if c1 == 0:
                cur = item_q(i1, 0)
            if u % NCS == 0:
                mrun = None
            mrun = stage1_chunk(u // NCS, cur[0], cur[1], c1, mrun)
            if u == NCS - 1:
                m_scr[0:8, :] = jnp.broadcast_to(jnp.max(mrun, axis=0, keepdims=True), (8, TQ))
        m_scr[8:16, :] = mrun
        for t in range(4):
            late_copy(t).wait()

    q0 = pl.multiple_of(step * TQ, TQ)
    q1 = pl.multiple_of(jnp.minimum(step + 1, NQ - 1) * TQ, TQ)
    low4q = lax.broadcasted_iota(jnp.int32, (8, TQ), 0) < 4

    def finish_pair(p, acc_e, acc_o):
        inv_e = 1.0 / acc_e[20:21, :]
        inv_o = 1.0 / acc_o[0:1, :]
        r0 = pl.multiple_of(p * 40, 8)
        ot_scr[pl.ds(r0, 16), :] = acc_e[0:16, :] * inv_e
        ot_scr[pl.ds(r0 + 16, 8), :] = jnp.where(low4q, acc_e[16:24, :] * inv_e, acc_o[0:8, :] * inv_o)
        ot_scr[pl.ds(r0 + 24, 16), :] = acc_o[8:24, :] * inv_o

    def body(it, carry):
        m, mrun = carry
        h0 = it * HPI
        wrap = h0 + HPI >= H
        qn = pl.multiple_of(jnp.where(wrap, q1, q0), TQ)
        hn = jnp.where(wrap, 0, h0 + HPI)
        fc = F // (H // HPI)
        nsub = fc // FSUB
        hidden = {}

        def ffn_up(j):
            c0 = pl.multiple_of(it * fc + j * FSUB, 128)
            xn = xn_scr[pl.ds(q0, TQ), :]
            g = jnp.dot(xn, wg_ref[:, pl.ds(c0, FSUB)], preferred_element_type=F32)
            u = jnp.dot(xn, wu_ref[:, pl.ds(c0, FSUB)], preferred_element_type=F32)
            hidden[j] = (g * jax.nn.sigmoid(g) * u).astype(BF16)

        def ffn_down(j):
            c0 = pl.multiple_of(it * fc + j * FSUB, 128)
            part = jnp.dot(hidden.pop(j), wd_ref[pl.ds(c0, FSUB), :], preferred_element_type=F32)
            if j == 0:
                prev = jnp.where(it == 0, x_ref[pl.ds(q0, TQ), :].astype(F32), y_scr[...])
            else:
                prev = y_scr[...]
            y_scr[...] = prev + part

        total = HPI * NCK
        ffn_at = {}
        for j in range(nsub):
            ffn_at[(2 * j) * total // (2 * nsub)] = (ffn_up, j)
            ffn_at[(2 * j + 1) * total // (2 * nsub)] = (ffn_down, j)

        m_next = None
        accs = []
        parts = []
        acc = None
        cur = None
        for t in range(total):
            if t in ffn_at:
                ffn_at[t][0](ffn_at[t][1])
            u = t + NCS + LEAD
            i1, c1 = divmod(u, NCK)
            if cur is None or c1 == 0:
                cur = item_q(h0 + i1, q0) if i1 < HPI else item_q(hn + (i1 - HPI), qn)
            if u % NCS == 0:
                mrun = None
            mrun = stage1_chunk(u // NCS, cur[0], cur[1], c1, mrun)
            if u % NCS == NCS - 1:
                m_next = jnp.max(mrun, axis=0, keepdims=True)
            i2, c2 = divmod(t, NCK)
            acc = stage2_chunk(t // NCS, h0 + i2, m, c2, m_scr[16:40, :] if t % NCS == 0 else acc)
            if t % NCS == NCS - 1:
                parts.append((m, acc))
                m = m_next
            if c2 == NCK - 1:
                mt = parts[0][0]
                for pm, _ in parts[1:]:
                    mt = jnp.maximum(mt, pm)
                tot = None
                for pm, pa in parts:
                    term = pa if len(parts) == 1 else pa * jnp.exp2(pm - mt)
                    tot = term if tot is None else tot + term
                parts = []
                accs.append(tot)
                if i2 % 2 == 1:
                    finish_pair((h0 + i2) // 2, accs[-2], accs[-1])
        return m, mrun

    m_fin, mrun_fin = lax.fori_loop(0, H // HPI, body, (m_scr[0:1, :], m_scr[8:16, :]))
    m_scr[0:8, :] = jnp.broadcast_to(m_fin, (8, TQ))
    m_scr[8:16, :] = mrun_fin

    @pl.when(step > 0)
    def _():
        for j in range(TQ // TO):
            o_copy(j, q0 - TQ).wait()

    for j in range(TQ // TO):
        o = ot_scr[:, j * TO:(j + 1) * TO].T.astype(BF16)
        attn = jnp.dot(o, wo_ref[...], preferred_element_type=F32)
        o_scr[j * TO:(j + 1) * TO, :] = (y_scr[j * TO:(j + 1) * TO, :] + attn).astype(BF16)
        o_copy(j, q0).start()

    @pl.when(step == NQ - 1)
    def _():
        for j in range(TQ // TO):
            o_copy(j, q0).wait()


@jax.jit
def pallas_parallel_sum__mha_block__swiglu_ffn__prompt_kernel(
    A_x: jax.Array,
    A_wqkv: jax.Array,
    A_wo: jax.Array,
    B_x: jax.Array,
    B_w_gate: jax.Array,
    B_w_up: jax.Array,
    B_w_down: jax.Array,
):
    del B_x
    x = A_x.reshape(S, D)
    hbm = pl.BlockSpec(memory_space=pl.ANY)
    out = pl.pallas_call(
        _kernel,
        grid=(NQ,),
        in_specs=[hbm] * 6,
        out_specs=hbm,
        out_shape=jax.ShapeDtypeStruct((S, D), A_x.dtype),
        scratch_shapes=[
            pltpu.VMEM((S, D), BF16),
            pltpu.VMEM((D, 3 * D), BF16),
            pltpu.VMEM((D, D), BF16),
            pltpu.VMEM((D, F), BF16),
            pltpu.VMEM((D, F), BF16),
            pltpu.VMEM((F, D), BF16),
            pltpu.SemaphoreType.DMA((NR + 7,)),
            pltpu.VMEM((S, D), BF16),
            pltpu.VMEM((NGX, S, 128), BF16),
            pltpu.VMEM((NGX, S, 128), BF16),
            pltpu.VMEM((H * 24, S), F32),
            pltpu.VMEM((2, S // NSP, TQ), F32),
            pltpu.VMEM((D, TQ), F32),
            pltpu.VMEM((40, TQ), F32),
            pltpu.VMEM((TQ, D), F32),
            pltpu.VMEM((TQ, D), BF16),
            pltpu.SemaphoreType.DMA((TQ // TO,)),
        ],
        compiler_params=pltpu.CompilerParams(
            dimension_semantics=("arbitrary",),
            vmem_limit_bytes=100 * 1024 * 1024,
        ),
    )(x, A_wqkv, A_wo, B_w_gate, B_w_up, B_w_down)
    return out.reshape(1, S, D)
```

```python
import math

import jax
import jax.numpy as jnp
from jax import lax
import jax.experimental.pallas as pl
import jax.experimental.pallas.tpu as pltpu

S, D, H, DH, F = 2048, 640, 32, 20, 1536
TQ = 512
TK = 128
NV = 8
TR = 256
TO = 128
HPI = 8
NSP = 4
LEAD = 1
NCH = 3
FSUB = 384
NG = D // 128
NGX = 2 * NG - 1
NQ = S // TQ
NR = S // TR
NCK = S // TK
NCS = NCK // NSP
EPS = 1e-5
QSCALE = (DH ** -0.5) * math.log2(math.e)
NT = (((1,), (1,)), ((), ()))
F32 = jnp.float32
BF16 = jnp.bfloat16
U32 = jnp.uint32


def _kernel(x_hbm, wqkv_hbm, wo_hbm, wg_hbm, wu_hbm, wd_hbm, o_hbm,
            x_ref, wqkv_ref, wo_ref, wg_ref, wu_ref, wd_ref, sems,
            xn_scr, q_scr, k_scr, vt_scr, s2_scr, ot_scr, m_scr, y_scr, o_scr, osems,
            qt_scr, kb_scr, kw_scr):
    step = pl.program_id(0)
    lane_q = lax.broadcasted_iota(jnp.int32, (TQ, 128), 1)

    def item_q(h, qrow):
        a = h * DH
        g = a // 128
        lo = a % 128
        gx = jnp.where(lo > 128 - DH, g + NG, g)
        rel = (lane_q - lo) & 127
        q = q_scr[gx, pl.ds(qrow, TQ), :]
        return gx, jnp.where(rel < DH, q.astype(F32), 0.0).astype(BF16)

    def vpu_scores(h, parity, qtile, c):
        ncc = TQ // 128
        qi = (h // 2) * NQ + qtile
        kr = pl.multiple_of(h * (DH * NV), NV)
        accs = [None] * NCH
        for d in range(DH):
            row = parity * DH + d
            qb = jnp.concatenate(
                [jnp.broadcast_to(qt_scr[qi, row:row + 1, cc * 128:(cc + 1) * 128], (NV, 128))
                 for cc in range(ncc)], axis=1)
            kb = kb_scr[c, pl.ds(kr + d * NV, NV), :]
            t = jnp.concatenate([kb] * ncc, axis=1) * qb
            j = d % NCH
            accs[j] = t if accs[j] is None else accs[j] + t
        acc = accs[0]
        for a in accs[1:]:
            acc = acc + a
        return acc

    def stage1_chunk(part, gx, qm, c, mrun, vinfo=None):
        r0 = (c % NCS) * TK
        nm = TK
        if vinfo is not None:
            nm = TK - NV
            if mrun is None:
                mrun = m_scr[40:48, :]
            v = vpu_scores(*vinfo, c)
            s2_scr[part % 2, r0 + nm:r0 + TK, :] = v
            mrun = jnp.maximum(mrun, v)
        s = lax.dot_general(k_scr[gx, c * TK:c * TK + nm, :], qm, NT, preferred_element_type=F32)
        s2_scr[part % 2, r0:r0 + nm, :] = s
        cm = jnp.max(s.reshape(nm // 8, 8, TQ), axis=0)
        return cm if mrun is None else jnp.maximum(mrun, cm)

    def stage2_chunk(part, h, m, c, acc):
        r0 = (c % NCS) * TK
        p = jnp.exp2(s2_scr[part % 2, r0:r0 + TK, :] - m).astype(BF16)
        vt = vt_scr[pl.ds(pl.multiple_of(h * 24, 8), 24), c * TK:(c + 1) * TK]
        return acc + jnp.dot(vt, p, preferred_element_type=F32)

    def x_copy(r):
        rows = pl.ds(pl.multiple_of(r * TR, TR), TR)
        return pltpu.make_async_copy(x_hbm.at[rows, :], x_ref.at[rows, :], sems.at[r])

    def w_copy(t):
        cols = pl.ds(t * D, D)
        return pltpu.make_async_copy(wqkv_hbm.at[:, cols], wqkv_ref.at[:, cols], sems.at[NR + t])

    late = ((wg_hbm, wg_ref), (wu_hbm, wu_ref), (wd_hbm, wd_ref), (wo_hbm, wo_ref))

    def late_copy(t):
        return pltpu.make_async_copy(late[t][0], late[t][1], sems.at[NR + 3 + t])

    def o_copy(j, row0):
        dst = pl.ds(pl.multiple_of(row0 + j * TO, TO), TO)
        return pltpu.make_async_copy(o_scr.at[pl.ds(j * TO, TO), :], o_hbm.at[dst, :], osems.at[j])

    @pl.when(step == 0)
    def _():
        x_copy(0).start()
        x_copy(1).start()
        w_copy(1).start()
        m_scr[16:40, :] = jnp.zeros((24, TQ), F32)
        m_scr[40:48, :] = jnp.full((8, TQ), -jnp.inf, F32)
        y_scr[...] = jnp.zeros((TQ, D), F32)

        upper = lax.broadcasted_iota(jnp.int32, (TR, 128), 1) >= 64
        low4 = lax.broadcasted_iota(jnp.int32, (8, TR), 0) < 4

        def row0(r):
            return r * TR if isinstance(r, int) else pl.multiple_of(r * TR, TR)

        def layernorm(r):
            rows = pl.ds(row0(r), TR)
            x = x_ref[rows, :].astype(F32)
            mu = jnp.mean(x, axis=-1, keepdims=True)
            xc = x - mu
            var = jnp.mean(xc * xc, axis=-1, keepdims=True)
            xn_scr[rows, :] = (xc * lax.rsqrt(var + EPS)).astype(BF16)

        def v_part(r):
            rows = pl.ds(row0(r), TR)
            vt = jnp.dot(xn_scr[rows, :], wqkv_ref[:, 2 * D:3 * D], preferred_element_type=F32).T
            for p in range(H // 2):
                mid = vt[40 * p + 16:40 * p + 24, :]
                vt_scr[48 * p:48 * p + 16, rows] = vt[40 * p:40 * p + 16, :]
                vt_scr[48 * p + 16:48 * p + 24, rows] = jnp.where(low4, mid, 1.0)
                vt_scr[48 * p + 24:48 * p + 32, rows] = jnp.where(low4, 1.0, mid)
                vt_scr[48 * p + 32:48 * p + 48, rows] = vt[40 * p + 24:40 * p + 40, :]

        def qk_part(r, t):
            rows = pl.ds(row0(r), TR)
            dst = (q_scr, k_scr)[t]
            y = jnp.dot(xn_scr[rows, :], wqkv_ref[:, t * D:(t + 1) * D], preferred_element_type=F32)
            if t == 0:
                y = y * QSCALE
            gs = [y[:, g * 128:(g + 1) * 128] for g in range(NG)]
            for g in range(NG):
                dst[g, rows, :] = gs[g].astype(dst.dtype)
            for g in range(NG - 1):
                dst[NG + g, rows, :] = jnp.where(upper, gs[g], gs[g + 1]).astype(dst.dtype)
            if t == 0:
                yt = y.astype(BF16).astype(F32).T
                qtile = r // (TQ // TR)
                cols = pl.ds(row0(r % (TQ // TR)), TR)
                for p in range(H // 2):
                    qt_scr[p * NQ + qtile, :, cols] = yt[40 * p:40 * p + 40, :]
            else:
                ka = y[TK - NV:TK, :].astype(BF16).astype(F32)
                kc = y[2 * TK - NV:2 * TK, :].astype(BF16).astype(F32)
                kw_scr[r] = pltpu.bitcast(ka, U32) | (pltpu.bitcast(kc, U32) >> 16)

        def kb_part(r, j0=0, j1=D):
            w = kw_scr[r]
            for j in range(j0, j1):
                bc = jnp.broadcast_to(w[:, j:j + 1], (NV, 128))
                kb_scr[2 * r, j * NV:(j + 1) * NV, :] = pltpu.bitcast(bc & U32(0xFFFF0000), F32)
                kb_scr[2 * r + 1, j * NV:(j + 1) * NV, :] = pltpu.bitcast(bc << 16, F32)

        x_copy(0).wait()
        w_copy(2).start()
        x_copy(2).start()
        w_copy(0).start()
        layernorm(0)
        x_copy(1).wait()
        layernorm(1)
        w_copy(1).wait()
        qk_part(0, 1)
        qk_part(1, 1)
        w_copy(2).wait()
        x_copy(2).wait()
        for r in range(3, NR):
            x_copy(r).start()
        layernorm(2)
        v_part(0)
        w_copy(0).wait()
        for t in range(4):
            late_copy(t).start()

        def rows_body(r, carry):
            @pl.when(r + 3 < NR)
            def _():
                x_copy(r + 3).wait()
            kb_part(r, 0, 214)
            qk_part(r, 0)
            kb_part(r, 214, 427)
            v_part(r + 1)
            kb_part(r, 427, D)
            qk_part(r + 2, 1)
            layernorm(jnp.where(r + 3 < NR, r + 3, 0))
            return carry

        lax.fori_loop(0, NR - 2, rows_body, 0)
        kb_part(NR - 2)
        qk_part(NR - 2, 0)
        kb_part(NR - 1)
        v_part(NR - 1)
        qk_part(NR - 1, 0)

        gx, qm = item_q(0, 0)
        mrun = None
        for c in range(NCS + LEAD):
            if c == NCS:
                m_scr[0:8, :] = jnp.broadcast_to(jnp.max(mrun, axis=0, keepdims=True), (8, TQ))
                mrun = None
            mrun = stage1_chunk(c // NCS, gx, qm, c, mrun)
        m_scr[8:16, :] = mrun
        for t in range(4):
            late_copy(t).wait()

    q0 = pl.multiple_of(step * TQ, TQ)
    low4q = lax.broadcasted_iota(jnp.int32, (8, TQ), 0) < 4

    def finish_pair(p, acc_e, acc_o):
        inv_e = 1.0 / acc_e[20:21, :]
        inv_o = 1.0 / acc_o[0:1, :]
        r0 = pl.multiple_of(p * 40, 8)
        ot_scr[pl.ds(r0, 16), :] = acc_e[0:16, :] * inv_e
        ot_scr[pl.ds(r0 + 16, 8), :] = jnp.where(low4q, acc_e[16:24, :] * inv_e, acc_o[0:8, :] * inv_o)
        ot_scr[pl.ds(r0 + 24, 16), :] = acc_o[8:24, :] * inv_o

    def body(it, carry):
        m, mrun = carry
        h0 = it * HPI
        wrap = h0 + HPI >= H
        tn = jnp.where(wrap, jnp.minimum(step + 1, NQ - 1), step)
        hn = jnp.where(wrap, 0, h0 + HPI)
        fc = F // (H // HPI)
        nsub = fc // FSUB
        hidden = {}

        def ffn_up(j):
            c0 = pl.multiple_of(it * fc + j * FSUB, 128)
            xn = xn_scr[pl.ds(q0, TQ), :]
            g = jnp.dot(xn, wg_ref[:, pl.ds(c0, FSUB)], preferred_element_type=F32)
            u = jnp.dot(xn, wu_ref[:, pl.ds(c0, FSUB)], preferred_element_type=F32)
            hidden[j] = (g * jax.nn.sigmoid(g) * u).astype(BF16)

        def ffn_down(j):
            c0 = pl.multiple_of(it * fc + j * FSUB, 128)
            part = jnp.dot(hidden.pop(j), wd_ref[pl.ds(c0, FSUB), :], preferred_element_type=F32)
            if j == 0:
                prev = jnp.where(it == 0, x_ref[pl.ds(q0, TQ), :].astype(F32), y_scr[...])
            else:
                prev = y_scr[...]
            y_scr[...] = prev + part

        total = HPI * NCK
        ffn_at = {}
        for j in range(nsub):
            ffn_at[(2 * j) * total // (2 * nsub)] = (ffn_up, j)
            ffn_at[(2 * j + 1) * total // (2 * nsub)] = (ffn_down, j)

        m_next = None
        accs = []
        parts = []
        acc = None
        cur = None
        for t in range(total):
            if t in ffn_at:
                ffn_at[t][0](ffn_at[t][1])
            u = t + NCS + LEAD
            i1, c1 = divmod(u, NCK)
            if cur is None or c1 == 0:
                if i1 < HPI:
                    cur = item_q(h0 + i1, q0)
                    vinfo = (h0 + i1, i1 % 2, step)
                else:
                    cur = item_q(hn + (i1 - HPI), pl.multiple_of(tn * TQ, TQ))
                    vinfo = (hn + (i1 - HPI), i1 % 2, tn)
            if u % NCS == 0:
                mrun = None
            mrun = stage1_chunk(u // NCS, cur[0], cur[1], c1, mrun, vinfo)
            if u % NCS == NCS - 1:
                m_next = jnp.max(mrun, axis=0, keepdims=True)
            i2, c2 = divmod(t, NCK)
            acc = stage2_chunk(t // NCS, h0 + i2, m, c2, m_scr[16:40, :] if t % NCS == 0 else acc)
            if t % NCS == NCS - 1:
                parts.append((m, acc))
                m = m_next
            if c2 == NCK - 1:
                mt = parts[0][0]
                for pm, _ in parts[1:]:
                    mt = jnp.maximum(mt, pm)
                tot = None
                for pm, pa in parts:
                    term = pa * jnp.exp2(pm - mt)
                    tot = term if tot is None else tot + term
                parts = []
                accs.append(tot)
                if i2 % 2 == 1:
                    finish_pair((h0 + i2) // 2, accs[-2], accs[-1])
        return m, mrun

    m_fin, mrun_fin = lax.fori_loop(0, H // HPI, body, (m_scr[0:1, :], m_scr[8:16, :]))
    m_scr[0:8, :] = jnp.broadcast_to(m_fin, (8, TQ))
    m_scr[8:16, :] = mrun_fin

    @pl.when(step > 0)
    def _():
        for j in range(TQ // TO):
            o_copy(j, q0 - TQ).wait()

    for j in range(TQ // TO):
        o = ot_scr[:, j * TO:(j + 1) * TO].T.astype(BF16)
        attn = jnp.dot(o, wo_ref[...], preferred_element_type=F32)
        o_scr[j * TO:(j + 1) * TO, :] = (y_scr[j * TO:(j + 1) * TO, :] + attn).astype(BF16)
        o_copy(j, q0).start()

    @pl.when(step == NQ - 1)
    def _():
        for j in range(TQ // TO):
            o_copy(j, q0).wait()


@jax.jit
def pallas_parallel_sum__mha_block__swiglu_ffn__prompt_kernel(
    A_x: jax.Array,
    A_wqkv: jax.Array,
    A_wo: jax.Array,
    B_x: jax.Array,
    B_w_gate: jax.Array,
    B_w_up: jax.Array,
    B_w_down: jax.Array,
):
    del B_x
    x = A_x.reshape(S, D)
    hbm = pl.BlockSpec(memory_space=pl.ANY)
    out = pl.pallas_call(
        _kernel,
        grid=(NQ,),
        in_specs=[hbm] * 6,
        out_specs=hbm,
        out_shape=jax.ShapeDtypeStruct((S, D), A_x.dtype),
        scratch_shapes=[
            pltpu.VMEM((S, D), BF16),
            pltpu.VMEM((D, 3 * D), BF16),
            pltpu.VMEM((D, D), BF16),
            pltpu.VMEM((D, F), BF16),
            pltpu.VMEM((D, F), BF16),
            pltpu.VMEM((F, D), BF16),
            pltpu.SemaphoreType.DMA((NR + 7,)),
            pltpu.VMEM((S, D), BF16),
            pltpu.VMEM((NGX, S, 128), BF16),
            pltpu.VMEM((NGX, S, 128), F32),
            pltpu.VMEM((H * 24, S), F32),
            pltpu.VMEM((2, S // NSP, TQ), F32),
            pltpu.VMEM((D, TQ), F32),
            pltpu.VMEM((48, TQ), F32),
            pltpu.VMEM((TQ, D), F32),
            pltpu.VMEM((TQ, D), BF16),
            pltpu.SemaphoreType.DMA((TQ // TO,)),
            pltpu.VMEM((H // 2 * NQ, 2 * DH, TQ), F32),
            pltpu.VMEM((NCK, D * NV, 128), F32),
            pltpu.VMEM((NR, NV, D), U32),
        ],
        compiler_params=pltpu.CompilerParams(
            dimension_semantics=("arbitrary",),
            vmem_limit_bytes=112 * 1024 * 1024,
        ),
    )(x, A_wqkv, A_wo, B_w_gate, B_w_up, B_w_down)
    return out.reshape(1, S, D)
```

```python
import math

import jax
import jax.numpy as jnp
from jax import lax
import jax.experimental.pallas as pl
import jax.experimental.pallas.tpu as pltpu

S, D, H, DH, F = 2048, 640, 32, 20, 1536
TQ = 512
TK = 128
NV = 8
TR = 256
TO = 128
HPI = 8
NSP = 4
LEAD = 1
NCH = 3
FSUB = 384
NG = D // 128
NGX = 2 * NG - 1
NQ = S // TQ
NR = S // TR
NCK = S // TK
NCS = NCK // NSP
EPS = 1e-5
QSCALE = (DH ** -0.5) * math.log2(math.e)
NT = (((1,), (1,)), ((), ()))
F32 = jnp.float32
BF16 = jnp.bfloat16
U32 = jnp.uint32


def _kernel(x_hbm, wqkv_hbm, wo_hbm, wg_hbm, wu_hbm, wd_hbm, o_hbm,
            x_ref, wqkv_ref, wo_ref, wg_ref, wu_ref, wd_ref, sems,
            xn_scr, q_scr, k_scr, vt_scr, s2_scr, ot_scr, m_scr, y_scr, o_scr, osems,
            qt_scr, kb_scr, kw_scr):
    step = pl.program_id(0)
    lane_q = lax.broadcasted_iota(jnp.int32, (TQ, 128), 1)

    def item_q(h, qrow):
        a = h * DH
        g = a // 128
        lo = a % 128
        gx = jnp.where(lo > 128 - DH, g + NG, g)
        rel = (lane_q - lo) & 127
        q = q_scr[gx, pl.ds(qrow, TQ), :]
        return gx, jnp.where(rel < DH, q.astype(F32), 0.0).astype(BF16)

    def vpu_scores(h, parity, qtile, c):
        ncc = TQ // 128
        qi = (h // 2) * NQ + qtile
        kr = pl.multiple_of(h * (DH * NV), NV)
        accs = [None] * NCH
        for d in range(DH):
            row = parity * DH + d
            qb = jnp.concatenate(
                [jnp.broadcast_to(qt_scr[qi, row:row + 1, cc * 128:(cc + 1) * 128], (NV, 128))
                 for cc in range(ncc)], axis=1)
            kb = kb_scr[c, pl.ds(kr + d * NV, NV), :]
            t = jnp.concatenate([kb] * ncc, axis=1) * qb
            j = d % NCH
            accs[j] = t if accs[j] is None else accs[j] + t
        acc = accs[0]
        for a in accs[1:]:
            acc = acc + a
        return acc

    def stage1_chunk(part, gx, qm, c, mrun, vinfo):
        r0 = (c % NCS) * TK
        nm = TK - 2 * NV if c % 2 == 0 else TK
        if mrun is None:
            mrun = m_scr[40:48, :]
        v = vpu_scores(*vinfo, c)
        rv = ((c % NCS) // 2 * 2 + 1) * TK - 2 * NV + (c % 2) * NV
        s2_scr[part % 2, rv:rv + NV, :] = v
        s = lax.dot_general(k_scr[gx, c * TK:c * TK + nm, :], qm, NT, preferred_element_type=F32)
        s2_scr[part % 2, r0:r0 + nm, :] = s
        mrun = jnp.maximum(mrun, v)
        return jnp.maximum(mrun, jnp.max(s.reshape(nm // 8, 8, TQ), axis=0))

    def stage2_chunk(part, h, m, c, acc):
        r0 = (c % NCS) * TK
        p = jnp.exp2(s2_scr[part % 2, r0:r0 + TK, :] - m).astype(BF16)
        vt = vt_scr[pl.ds(pl.multiple_of(h * 24, 8), 24), c * TK:(c + 1) * TK]
        return acc + jnp.dot(vt, p, preferred_element_type=F32)

    def x_copy(r):
        rows = pl.ds(pl.multiple_of(r * TR, TR), TR)
        return pltpu.make_async_copy(x_hbm.at[rows, :], x_ref.at[rows, :], sems.at[r])

    def w_copy(t):
        cols = pl.ds(t * D, D)
        return pltpu.make_async_copy(wqkv_hbm.at[:, cols], wqkv_ref.at[:, cols], sems.at[NR + t])

    late = ((wg_hbm, wg_ref), (wu_hbm, wu_ref), (wd_hbm, wd_ref), (wo_hbm, wo_ref))

    def late_copy(t):
        return pltpu.make_async_copy(late[t][0], late[t][1], sems.at[NR + 3 + t])

    def o_copy(j, row0):
        dst = pl.ds(pl.multiple_of(row0 + j * TO, TO), TO)
        return pltpu.make_async_copy(o_scr.at[pl.ds(j * TO, TO), :], o_hbm.at[dst, :], osems.at[j])

    @pl.when(step == 0)
    def _():
        x_copy(0).start()
        x_copy(1).start()
        w_copy(1).start()
        m_scr[16:40, :] = jnp.zeros((24, TQ), F32)
        m_scr[40:48, :] = jnp.full((8, TQ), -jnp.inf, F32)
        y_scr[...] = jnp.zeros((TQ, D), F32)

        upper = lax.broadcasted_iota(jnp.int32, (TR, 128), 1) >= 64
        low4 = lax.broadcasted_iota(jnp.int32, (8, TR), 0) < 4

        def row0(r):
            return r * TR if isinstance(r, int) else pl.multiple_of(r * TR, TR)

        def layernorm(r):
            rows = pl.ds(row0(r), TR)
            x = x_ref[rows, :].astype(F32)
            mu = jnp.mean(x, axis=-1, keepdims=True)
            xc = x - mu
            var = jnp.mean(xc * xc, axis=-1, keepdims=True)
            xn_scr[rows, :] = (xc * lax.rsqrt(var + EPS)).astype(BF16)

        def v_part(r):
            rows = pl.ds(row0(r), TR)
            vt = jnp.dot(xn_scr[rows, :], wqkv_ref[:, 2 * D:3 * D], preferred_element_type=F32).T
            for p in range(H // 2):
                mid = vt[40 * p + 16:40 * p + 24, :]
                vt_scr[48 * p:48 * p + 16, rows] = vt[40 * p:40 * p + 16, :]
                vt_scr[48 * p + 16:48 * p + 24, rows] = jnp.where(low4, mid, 1.0)
                vt_scr[48 * p + 24:48 * p + 32, rows] = jnp.where(low4, 1.0, mid)
                vt_scr[48 * p + 32:48 * p + 48, rows] = vt[40 * p + 24:40 * p + 40, :]

        def qk_part(r, t):
            rows = pl.ds(row0(r), TR)
            dst = (q_scr, k_scr)[t]
            y = jnp.dot(xn_scr[rows, :], wqkv_ref[:, t * D:(t + 1) * D], preferred_element_type=F32)
            if t == 0:
                y = y * QSCALE
            gs = [y[:, g * 128:(g + 1) * 128] for g in range(NG)]
            for g in range(NG):
                dst[g, rows, :] = gs[g].astype(BF16)
            for g in range(NG - 1):
                dst[NG + g, rows, :] = jnp.where(upper, gs[g], gs[g + 1]).astype(BF16)
            if t == 0:
                yt = y.astype(BF16).astype(F32).T
                qtile = r // (TQ // TR)
                cols = pl.ds(row0(r % (TQ // TR)), TR)
                for p in range(H // 2):
                    qt_scr[p * NQ + qtile, :, cols] = yt[40 * p:40 * p + 40, :]
            else:
                ka = y[TK - 2 * NV:TK - NV, :].astype(BF16).astype(F32)
                kc = y[TK - NV:TK, :].astype(BF16).astype(F32)
                kw_scr[r] = pltpu.bitcast(ka, U32) | (pltpu.bitcast(kc, U32) >> 16)

        def kb_part(r, j0=0, j1=D):
            w = kw_scr[r]
            for j in range(j0, j1):
                bc = jnp.broadcast_to(w[:, j:j + 1], (NV, 128))
                kb_scr[2 * r, j * NV:(j + 1) * NV, :] = pltpu.bitcast(bc & U32(0xFFFF0000), F32)
                kb_scr[2 * r + 1, j * NV:(j + 1) * NV, :] = pltpu.bitcast(bc << 16, F32)

        x_copy(0).wait()
        w_copy(2).start()
        x_copy(2).start()
        w_copy(0).start()
        layernorm(0)
        x_copy(1).wait()
        layernorm(1)
        w_copy(1).wait()
        qk_part(0, 1)
        qk_part(1, 1)
        w_copy(2).wait()
        x_copy(2).wait()
        for r in range(3, NR):
            x_copy(r).start()
        layernorm(2)
        v_part(0)
        w_copy(0).wait()
        for t in range(4):
            late_copy(t).start()

        def rows_body(r, carry):
            @pl.when(r + 3 < NR)
            def _():
                x_copy(r + 3).wait()
            kb_part(r, 0, 214)
            qk_part(r, 0)
            kb_part(r, 214, 427)
            v_part(r + 1)
            kb_part(r, 427, D)
            qk_part(r + 2, 1)
            layernorm(jnp.where(r + 3 < NR, r + 3, 0))
            return carry

        lax.fori_loop(0, NR - 2, rows_body, 0)
        kb_part(NR - 2)
        qk_part(NR - 2, 0)
        kb_part(NR - 1)
        v_part(NR - 1)
        qk_part(NR - 1, 0)

        gx, qm = item_q(0, 0)
        mrun = None
        for c in range(NCS + LEAD):
            if c == NCS:
                m_scr[0:8, :] = jnp.broadcast_to(jnp.max(mrun, axis=0, keepdims=True), (8, TQ))
                mrun = None
            mrun = stage1_chunk(c // NCS, gx, qm, c, mrun, (0, 0, 0))
        m_scr[8:16, :] = mrun
        for t in range(4):
            late_copy(t).wait()

    q0 = pl.multiple_of(step * TQ, TQ)
    low4q = lax.broadcasted_iota(jnp.int32, (8, TQ), 0) < 4

    def finish_pair(p, acc_e, acc_o):
        inv_e = 1.0 / acc_e[20:21, :]
        inv_o = 1.0 / acc_o[0:1, :]
        r0 = pl.multiple_of(p * 40, 8)
        ot_scr[pl.ds(r0, 16), :] = acc_e[0:16, :] * inv_e
        ot_scr[pl.ds(r0 + 16, 8), :] = jnp.where(low4q, acc_e[16:24, :] * inv_e, acc_o[0:8, :] * inv_o)
        ot_scr[pl.ds(r0 + 24, 16), :] = acc_o[8:24, :] * inv_o

    def body(it, carry):
        m, mrun = carry
        h0 = it * HPI
        wrap = h0 + HPI >= H
        tn = jnp.where(wrap, jnp.minimum(step + 1, NQ - 1), step)
        hn = jnp.where(wrap, 0, h0 + HPI)
        fc = F // (H // HPI)
        nsub = fc // FSUB
        hidden = {}

        def ffn_up(j):
            c0 = pl.multiple_of(it * fc + j * FSUB, 128)
            xn = xn_scr[pl.ds(q0, TQ), :]
            g = jnp.dot(xn, wg_ref[:, pl.ds(c0, FSUB)], preferred_element_type=F32)
            u = jnp.dot(xn, wu_ref[:, pl.ds(c0, FSUB)], preferred_element_type=F32)
            hidden[j] = (g * jax.nn.sigmoid(g) * u).astype(BF16)

        def ffn_down(j):
            c0 = pl.multiple_of(it * fc + j * FSUB, 128)
            part = jnp.dot(hidden.pop(j), wd_ref[pl.ds(c0, FSUB), :], preferred_element_type=F32)
            if j == 0:
                prev = jnp.where(it == 0, x_ref[pl.ds(q0, TQ), :].astype(F32), y_scr[...])
            else:
                prev = y_scr[...]
            y_scr[...] = prev + part

        total = HPI * NCK
        ffn_at = {}
        for j in range(nsub):
            ffn_at[(2 * j) * total // (2 * nsub)] = (ffn_up, j)
            ffn_at[(2 * j + 1) * total // (2 * nsub)] = (ffn_down, j)

        m_next = None
        accs = []
        parts = []
        acc = None
        cur = None
        for t in range(total):
            if t in ffn_at:
                ffn_at[t][0](ffn_at[t][1])
            u = t + NCS + LEAD
            i1, c1 = divmod(u, NCK)
            if cur is None or c1 == 0:
                if i1 < HPI:
                    cur = item_q(h0 + i1, q0)
                    vinfo = (h0 + i1, i1 % 2, step)
                else:
                    cur = item_q(hn + (i1 - HPI), pl.multiple_of(tn * TQ, TQ))
                    vinfo = (hn + (i1 - HPI), i1 % 2, tn)
            if u % NCS == 0:
                mrun = None
            mrun = stage1_chunk(u // NCS, cur[0], cur[1], c1, mrun, vinfo)
            if u % NCS == NCS - 1:
                m_next = jnp.max(mrun, axis=0, keepdims=True)
            i2, c2 = divmod(t, NCK)
            acc = stage2_chunk(t // NCS, h0 + i2, m, c2, m_scr[16:40, :] if t % NCS == 0 else acc)
            if t % NCS == NCS - 1:
                parts.append((m, acc))
                m = m_next
            if c2 == NCK - 1:
                mt = parts[0][0]
                for pm, _ in parts[1:]:
                    mt = jnp.maximum(mt, pm)
                tot = None
                for pm, pa in parts:
                    term = pa * jnp.exp2(pm - mt)
                    tot = term if tot is None else tot + term
                parts = []
                accs.append(tot)
                if i2 % 2 == 1:
                    finish_pair((h0 + i2) // 2, accs[-2], accs[-1])
        return m, mrun

    m_fin, mrun_fin = lax.fori_loop(0, H // HPI, body, (m_scr[0:1, :], m_scr[8:16, :]))
    m_scr[0:8, :] = jnp.broadcast_to(m_fin, (8, TQ))
    m_scr[8:16, :] = mrun_fin

    @pl.when(step > 0)
    def _():
        for j in range(TQ // TO):
            o_copy(j, q0 - TQ).wait()

    for j in range(TQ // TO):
        o = ot_scr[:, j * TO:(j + 1) * TO].T.astype(BF16)
        attn = jnp.dot(o, wo_ref[...], preferred_element_type=F32)
        o_scr[j * TO:(j + 1) * TO, :] = (y_scr[j * TO:(j + 1) * TO, :] + attn).astype(BF16)
        o_copy(j, q0).start()

    @pl.when(step == NQ - 1)
    def _():
        for j in range(TQ // TO):
            o_copy(j, q0).wait()


@jax.jit
def pallas_parallel_sum__mha_block__swiglu_ffn__prompt_kernel(
    A_x: jax.Array,
    A_wqkv: jax.Array,
    A_wo: jax.Array,
    B_x: jax.Array,
    B_w_gate: jax.Array,
    B_w_up: jax.Array,
    B_w_down: jax.Array,
):
    del B_x
    x = A_x.reshape(S, D)
    hbm = pl.BlockSpec(memory_space=pl.ANY)
    out = pl.pallas_call(
        _kernel,
        grid=(NQ,),
        in_specs=[hbm] * 6,
        out_specs=hbm,
        out_shape=jax.ShapeDtypeStruct((S, D), A_x.dtype),
        scratch_shapes=[
            pltpu.VMEM((S, D), BF16),
            pltpu.VMEM((D, 3 * D), BF16),
            pltpu.VMEM((D, D), BF16),
            pltpu.VMEM((D, F), BF16),
            pltpu.VMEM((D, F), BF16),
            pltpu.VMEM((F, D), BF16),
            pltpu.SemaphoreType.DMA((NR + 7,)),
            pltpu.VMEM((S, D), BF16),
            pltpu.VMEM((NGX, S, 128), BF16),
            pltpu.VMEM((NGX, S, 128), BF16),
            pltpu.VMEM((H * 24, S), F32),
            pltpu.VMEM((2, S // NSP, TQ), F32),
            pltpu.VMEM((D, TQ), F32),
            pltpu.VMEM((48, TQ), F32),
            pltpu.VMEM((TQ, D), F32),
            pltpu.VMEM((TQ, D), BF16),
            pltpu.SemaphoreType.DMA((TQ // TO,)),
            pltpu.VMEM((H // 2 * NQ, 2 * DH, TQ), F32),
            pltpu.VMEM((NCK, D * NV, 128), F32),
            pltpu.VMEM((NR, NV, D), U32),
        ],
        compiler_params=pltpu.CompilerParams(
            dimension_semantics=("arbitrary",),
            vmem_limit_bytes=112 * 1024 * 1024,
        ),
    )(x, A_wqkv, A_wo, B_w_gate, B_w_up, B_w_down)
    return out.reshape(1, S, D)
```

```python
import math

import jax
import jax.numpy as jnp
from jax import lax
import jax.experimental.pallas as pl
import jax.experimental.pallas.tpu as pltpu

S, D, H, DH, F = 2048, 640, 32, 20, 1536
TQ = 512
TK = 128
NV = 8
TR = 256
TO = 128
HPI = 8
NSP = 4
LEAD = 1
NCH = 2
NG = D // 128
NGX = 2 * NG - 1
NQ = S // TQ
NR = S // TR
NCK = S // TK
NCS = NCK // NSP
EPS = 1e-5
QSCALE = (DH ** -0.5) * math.log2(math.e)
NT = (((1,), (1,)), ((), ()))
F32 = jnp.float32
BF16 = jnp.bfloat16
U32 = jnp.uint32


def _kernel(x_hbm, wqkv_hbm, wo_hbm, wg_hbm, wu_hbm, wd_hbm, o_hbm,
            x_ref, wqkv_ref, wo_ref, wg_ref, wu_ref, wd_ref, sems,
            xn_scr, q_scr, k_scr, vt_scr, s2_scr, ot_scr, m_scr, y_scr, o_scr, osems,
            qt_scr, kb_scr, kw_scr):
    step = pl.program_id(0)
    lane_q = lax.broadcasted_iota(jnp.int32, (TQ, 128), 1)

    def item_q(h, qrow):
        a = h * DH
        g = a // 128
        lo = a % 128
        gx = jnp.where(lo > 128 - DH, g + NG, g)
        rel = (lane_q - lo) & 127
        q = q_scr[gx, pl.ds(qrow, TQ), :]
        return gx, jnp.where(rel < DH, q.astype(F32), 0.0).astype(BF16)

    def vpu_scores(h, parity, qtile, c):
        ncc = TQ // 128
        qi = (h // 2) * NQ + qtile
        kr = pl.multiple_of(h * (DH * NV), NV)
        accs = [None] * NCH
        for d in range(DH):
            row = parity * DH + d
            qb = jnp.concatenate(
                [jnp.broadcast_to(qt_scr[qi, row:row + 1, cc * 128:(cc + 1) * 128], (NV, 128))
                 for cc in range(ncc)], axis=1)
            kb = kb_scr[c, pl.ds(kr + d * NV, NV), :]
            t = jnp.concatenate([kb] * ncc, axis=1) * qb
            j = d % NCH
            accs[j] = t if accs[j] is None else accs[j] + t
        acc = accs[0]
        for a in accs[1:]:
            acc = acc + a
        return acc

    def stage1_chunk(part, gx, qm, c, mrun, vinfo):
        r0 = (c % NCS) * TK
        nm = TK - 2 * NV if c % 2 == 0 else TK
        if mrun is None:
            mrun = m_scr[40:48, :]
        v = vpu_scores(*vinfo, c)
        rv = ((c % NCS) // 2 * 2 + 1) * TK - 2 * NV + (c % 2) * NV
        s2_scr[part % 2, rv:rv + NV, :] = v
        s = lax.dot_general(k_scr[gx, c * TK:c * TK + nm, :], qm, NT, preferred_element_type=F32)
        s2_scr[part % 2, r0:r0 + nm, :] = s
        mrun = jnp.maximum(mrun, v)
        return jnp.maximum(mrun, jnp.max(s.reshape(nm // 8, 8, TQ), axis=0))

    def stage2_chunk(part, h, m, c, acc):
        r0 = (c % NCS) * TK
        p = jnp.exp2(s2_scr[part % 2, r0:r0 + TK, :] - m).astype(BF16)
        vt = vt_scr[pl.ds(pl.multiple_of(h * 24, 8), 24), c * TK:(c + 1) * TK]
        return acc + jnp.dot(vt, p, preferred_element_type=F32)

    def x_copy(r):
        rows = pl.ds(pl.multiple_of(r * TR, TR), TR)
        return pltpu.make_async_copy(x_hbm.at[rows, :], x_ref.at[rows, :], sems.at[r])

    def w_copy(t):
        cols = pl.ds(t * D, D)
        return pltpu.make_async_copy(wqkv_hbm.at[:, cols], wqkv_ref.at[:, cols], sems.at[NR + t])

    late = ((wg_hbm, wg_ref), (wu_hbm, wu_ref), (wd_hbm, wd_ref), (wo_hbm, wo_ref))

    def late_copy(t):
        return pltpu.make_async_copy(late[t][0], late[t][1], sems.at[NR + 3 + t])

    def o_copy(j, row0):
        dst = pl.ds(pl.multiple_of(row0 + j * TO, TO), TO)
        return pltpu.make_async_copy(o_scr.at[pl.ds(j * TO, TO), :], o_hbm.at[dst, :], osems.at[j])

    @pl.when(step == 0)
    def _():
        x_copy(0).start()
        x_copy(1).start()
        w_copy(1).start()
        m_scr[16:40, :] = jnp.zeros((24, TQ), F32)
        m_scr[40:48, :] = jnp.full((8, TQ), -jnp.inf, F32)
        y_scr[...] = jnp.zeros((TQ, D), F32)

        upper = lax.broadcasted_iota(jnp.int32, (TR, 128), 1) >= 64
        low4 = lax.broadcasted_iota(jnp.int32, (8, TR), 0) < 4

        def row0(r):
            return r * TR if isinstance(r, int) else pl.multiple_of(r * TR, TR)

        def layernorm(r):
            rows = pl.ds(row0(r), TR)
            x = x_ref[rows, :].astype(F32)
            mu = jnp.mean(x, axis=-1, keepdims=True)
            xc = x - mu
            var = jnp.mean(xc * xc, axis=-1, keepdims=True)
            xn_scr[rows, :] = (xc * lax.rsqrt(var + EPS)).astype(BF16)

        def v_part(r):
            rows = pl.ds(row0(r), TR)
            vt = jnp.dot(xn_scr[rows, :], wqkv_ref[:, 2 * D:3 * D], preferred_element_type=F32).T
            for p in range(H // 2):
                mid = vt[40 * p + 16:40 * p + 24, :]
                vt_scr[48 * p:48 * p + 16, rows] = vt[40 * p:40 * p + 16, :]
                vt_scr[48 * p + 16:48 * p + 24, rows] = jnp.where(low4, mid, 1.0)
                vt_scr[48 * p + 24:48 * p + 32, rows] = jnp.where(low4, 1.0, mid)
                vt_scr[48 * p + 32:48 * p + 48, rows] = vt[40 * p + 24:40 * p + 40, :]

        def qk_part(r, t):
            rows = pl.ds(row0(r), TR)
            dst = (q_scr, k_scr)[t]
            y = jnp.dot(xn_scr[rows, :], wqkv_ref[:, t * D:(t + 1) * D], preferred_element_type=F32)
            if t == 0:
                y = y * QSCALE
            gs = [y[:, g * 128:(g + 1) * 128] for g in range(NG)]
            for g in range(NG):
                dst[g, rows, :] = gs[g].astype(BF16)
            for g in range(NG - 1):
                dst[NG + g, rows, :] = jnp.where(upper, gs[g], gs[g + 1]).astype(BF16)
            if t == 0:
                yt = y.astype(BF16).astype(F32).T
                qtile = r // (TQ // TR)
                cols = pl.ds(row0(r % (TQ // TR)), TR)
                for p in range(H // 2):
                    qt_scr[p * NQ + qtile, :, cols] = yt[40 * p:40 * p + 40, :]
            else:
                ka = y[TK - 2 * NV:TK - NV, :].astype(BF16).astype(F32)
                kc = y[TK - NV:TK, :].astype(BF16).astype(F32)
                kw_scr[r] = pltpu.bitcast(ka, U32) | (pltpu.bitcast(kc, U32) >> 16)

        def kb_part(r, j0=0, j1=D):
            w = kw_scr[r]
            for j in range(j0, j1):
                bc = jnp.broadcast_to(w[:, j:j + 1], (NV, 128))
                kb_scr[2 * r, j * NV:(j + 1) * NV, :] = pltpu.bitcast(bc & U32(0xFFFF0000), F32)
                kb_scr[2 * r + 1, j * NV:(j + 1) * NV, :] = pltpu.bitcast(bc << 16, F32)

        x_copy(0).wait()
        w_copy(2).start()
        x_copy(2).start()
        w_copy(0).start()
        layernorm(0)
        x_copy(1).wait()
        layernorm(1)
        w_copy(1).wait()
        qk_part(0, 1)
        qk_part(1, 1)
        w_copy(2).wait()
        x_copy(2).wait()
        for r in range(3, NR):
            x_copy(r).start()
        layernorm(2)
        v_part(0)
        w_copy(0).wait()
        for t in range(4):
            late_copy(t).start()

        def rows_body(r, carry):
            @pl.when(r + 3 < NR)
            def _():
                x_copy(r + 3).wait()
            kb_part(r, 0, 214)
            qk_part(r, 0)
            kb_part(r, 214, 427)
            v_part(r + 1)
            kb_part(r, 427, D)
            qk_part(r + 2, 1)
            layernorm(jnp.where(r + 3 < NR, r + 3, 0))
            return carry

        lax.fori_loop(0, NR - 2, rows_body, 0)
        kb_part(NR - 2)
        qk_part(NR - 2, 0)
        kb_part(NR - 1)
        v_part(NR - 1)
        qk_part(NR - 1, 0)

        gx, qm = item_q(0, 0)
        mrun = None
        for c in range(NCS + LEAD):
            if c == NCS:
                m_scr[0:8, :] = jnp.broadcast_to(jnp.max(mrun, axis=0, keepdims=True), (8, TQ))
                mrun = None
            mrun = stage1_chunk(c // NCS, gx, qm, c, mrun, (0, 0, 0))
        m_scr[8:16, :] = mrun
        for t in range(4):
            late_copy(t).wait()

    q0 = pl.multiple_of(step * TQ, TQ)
    low4q = lax.broadcasted_iota(jnp.int32, (8, TQ), 0) < 4

    def finish_pair(p, acc_e, acc_o):
        inv_e = 1.0 / acc_e[20:21, :]
        inv_o = 1.0 / acc_o[0:1, :]
        r0 = pl.multiple_of(p * 40, 8)
        ot_scr[pl.ds(r0, 16), :] = acc_e[0:16, :] * inv_e
        ot_scr[pl.ds(r0 + 16, 8), :] = jnp.where(low4q, acc_e[16:24, :] * inv_e, acc_o[0:8, :] * inv_o)
        ot_scr[pl.ds(r0 + 24, 16), :] = acc_o[8:24, :] * inv_o

    def body(it, carry):
        m, mrun = carry
        h0 = it * HPI
        wrap = h0 + HPI >= H
        tn = jnp.where(wrap, jnp.minimum(step + 1, NQ - 1), step)
        hn = jnp.where(wrap, 0, h0 + HPI)
        fc = F // (H // HPI)
        fcols = pl.ds(pl.multiple_of(it * fc, 128), fc)

        def ffn_up():
            xn = xn_scr[pl.ds(q0, TQ), :]
            g = jnp.dot(xn, wg_ref[:, fcols], preferred_element_type=F32)
            u = jnp.dot(xn, wu_ref[:, fcols], preferred_element_type=F32)
            return (g * jax.nn.sigmoid(g) * u).astype(BF16)

        def ffn_down(hidden):
            part = jnp.dot(hidden, wd_ref[fcols, :], preferred_element_type=F32)
            prev = jnp.where(it == 0, x_ref[pl.ds(q0, TQ), :].astype(F32), y_scr[...])
            y_scr[...] = prev + part

        m_next = None
        accs = []
        parts = []
        acc = None
        cur = None
        for t in range(HPI * NCK):
            if t == 0:
                hidden = ffn_up()
            elif t == 1:
                ffn_down(hidden)
            u = t + NCS + LEAD
            i1, c1 = divmod(u, NCK)
            if cur is None or c1 == 0:
                if i1 < HPI:
                    cur = item_q(h0 + i1, q0)
                    vinfo = (h0 + i1, i1 % 2, step)
                else:
                    cur = item_q(hn + (i1 - HPI), pl.multiple_of(tn * TQ, TQ))
                    vinfo = (hn + (i1 - HPI), i1 % 2, tn)
            if u % NCS == 0:
                mrun = None
            mrun = stage1_chunk(u // NCS, cur[0], cur[1], c1, mrun, vinfo)
            if u % NCS == NCS - 1:
                m_next = jnp.max(mrun, axis=0, keepdims=True)
            i2, c2 = divmod(t, NCK)
            acc = stage2_chunk(t // NCS, h0 + i2, m, c2, m_scr[16:40, :] if t % NCS == 0 else acc)
            if t % NCS == NCS - 1:
                parts.append((m, acc))
                m = m_next
            if c2 == NCK - 1:
                mt = parts[0][0]
                for pm, _ in parts[1:]:
                    mt = jnp.maximum(mt, pm)
                tot = None
                for pm, pa in parts:
                    term = pa * jnp.exp2(pm - mt)
                    tot = term if tot is None else tot + term
                parts = []
                accs.append(tot)
                if i2 % 2 == 1:
                    finish_pair((h0 + i2) // 2, accs[-2], accs[-1])
        return m, mrun

    m_fin, mrun_fin = lax.fori_loop(0, H // HPI, body, (m_scr[0:1, :], m_scr[8:16, :]))
    m_scr[0:8, :] = jnp.broadcast_to(m_fin, (8, TQ))
    m_scr[8:16, :] = mrun_fin

    @pl.when(step > 0)
    def _():
        for j in range(TQ // TO):
            o_copy(j, q0 - TQ).wait()

    for j in range(TQ // TO):
        o = ot_scr[:, j * TO:(j + 1) * TO].T.astype(BF16)
        attn = jnp.dot(o, wo_ref[...], preferred_element_type=F32)
        o_scr[j * TO:(j + 1) * TO, :] = (y_scr[j * TO:(j + 1) * TO, :] + attn).astype(BF16)
        o_copy(j, q0).start()

    @pl.when(step == NQ - 1)
    def _():
        for j in range(TQ // TO):
            o_copy(j, q0).wait()


@jax.jit
def pallas_parallel_sum__mha_block__swiglu_ffn__prompt_kernel(
    A_x: jax.Array,
    A_wqkv: jax.Array,
    A_wo: jax.Array,
    B_x: jax.Array,
    B_w_gate: jax.Array,
    B_w_up: jax.Array,
    B_w_down: jax.Array,
):
    del B_x
    x = A_x.reshape(S, D)
    hbm = pl.BlockSpec(memory_space=pl.ANY)
    out = pl.pallas_call(
        _kernel,
        grid=(NQ,),
        in_specs=[hbm] * 6,
        out_specs=hbm,
        out_shape=jax.ShapeDtypeStruct((S, D), A_x.dtype),
        scratch_shapes=[
            pltpu.VMEM((S, D), BF16),
            pltpu.VMEM((D, 3 * D), BF16),
            pltpu.VMEM((D, D), BF16),
            pltpu.VMEM((D, F), BF16),
            pltpu.VMEM((D, F), BF16),
            pltpu.VMEM((F, D), BF16),
            pltpu.SemaphoreType.DMA((NR + 7,)),
            pltpu.VMEM((S, D), BF16),
            pltpu.VMEM((NGX, S, 128), BF16),
            pltpu.VMEM((NGX, S, 128), BF16),
            pltpu.VMEM((H * 24, S), F32),
            pltpu.VMEM((2, S // NSP, TQ), F32),
            pltpu.VMEM((D, TQ), F32),
            pltpu.VMEM((48, TQ), F32),
            pltpu.VMEM((TQ, D), F32),
            pltpu.VMEM((TQ, D), BF16),
            pltpu.SemaphoreType.DMA((TQ // TO,)),
            pltpu.VMEM((H // 2 * NQ, 2 * DH, TQ), F32),
            pltpu.VMEM((NCK, D * NV, 128), F32),
            pltpu.VMEM((NR, NV, D), U32),
        ],
        compiler_params=pltpu.CompilerParams(
            dimension_semantics=("arbitrary",),
            vmem_limit_bytes=112 * 1024 * 1024,
        ),
    )(x, A_wqkv, A_wo, B_w_gate, B_w_up, B_w_down)
    return out.reshape(1, S, D)
```

```python
import math

import jax
import jax.numpy as jnp
from jax import lax
import jax.experimental.pallas as pl
import jax.experimental.pallas.tpu as pltpu

S, D, H, DH, F = 2048, 640, 32, 20, 1536
TQ = 512
TK = 128
NV = 8
TR = 256
TO = 128
HPI = 8
NSP = 4
LEAD = 1
FL = 128
NCH = 2
NG = D // 128
NGX = 2 * NG - 1
NQ = S // TQ
NR = S // TR
NCK = S // TK
NCS = NCK // NSP
EPS = 1e-5
QSCALE = (DH ** -0.5) * math.log2(math.e)
NT = (((1,), (1,)), ((), ()))
F32 = jnp.float32
BF16 = jnp.bfloat16
U32 = jnp.uint32


def _kernel(x_hbm, wqkv_hbm, wo_hbm, wg_hbm, wu_hbm, wd_hbm, o_hbm,
            x_ref, wqkv_ref, wo_ref, wg_ref, wu_ref, wd_ref, sems,
            xn_scr, q_scr, k_scr, vt_scr, s2_scr, ot_scr, m_scr, y_scr, o_scr, osems,
            qt_scr, kb_scr, kw_scr):
    step = pl.program_id(0)
    lane_q = lax.broadcasted_iota(jnp.int32, (TQ, 128), 1)

    def item_q(h, qrow):
        a = h * DH
        g = a // 128
        lo = a % 128
        gx = jnp.where(lo > 128 - DH, g + NG, g)
        rel = (lane_q - lo) & 127
        q = q_scr[gx, pl.ds(qrow, TQ), :]
        return gx, jnp.where(rel < DH, q.astype(F32), 0.0).astype(BF16)

    def vpu_scores(h, parity, qtile, c):
        ncc = TQ // 128
        qi = (h // 2) * NQ + qtile
        kr = pl.multiple_of(h * (DH * NV), NV)
        accs = [None] * NCH
        for d in range(DH):
            row = parity * DH + d
            qb = jnp.concatenate(
                [jnp.broadcast_to(qt_scr[qi, row:row + 1, cc * 128:(cc + 1) * 128], (NV, 128))
                 for cc in range(ncc)], axis=1)
            kb = kb_scr[c, pl.ds(kr + d * NV, NV), :]
            t = jnp.concatenate([kb] * ncc, axis=1) * qb
            j = d % NCH
            accs[j] = t if accs[j] is None else accs[j] + t
        acc = accs[0]
        for a in accs[1:]:
            acc = acc + a
        return acc

    def stage1_chunk(part, gx, qm, c, mrun, vinfo):
        r0 = (c % NCS) * TK
        nm = TK - 2 * NV if c % 2 == 0 else TK
        if mrun is None:
            mrun = m_scr[40:48, :]
        v = vpu_scores(*vinfo, c)
        rv = ((c % NCS) // 2 * 2 + 1) * TK - 2 * NV + (c % 2) * NV
        s2_scr[part % 2, rv:rv + NV, :] = v
        s = lax.dot_general(k_scr[gx, c * TK:c * TK + nm, :], qm, NT, preferred_element_type=F32)
        s2_scr[part % 2, r0:r0 + nm, :] = s
        mrun = jnp.maximum(mrun, v)
        return jnp.maximum(mrun, jnp.max(s.reshape(nm // 8, 8, TQ), axis=0))

    def stage2_chunk(part, h, m, c, acc):
        r0 = (c % NCS) * TK
        p = jnp.exp2(s2_scr[part % 2, r0:r0 + TK, :] - m).astype(BF16)
        vt = vt_scr[pl.ds(pl.multiple_of(h * 24, 8), 24), c * TK:(c + 1) * TK]
        return acc + jnp.dot(vt, p, preferred_element_type=F32)

    def x_copy(r):
        rows = pl.ds(pl.multiple_of(r * TR, TR), TR)
        return pltpu.make_async_copy(x_hbm.at[rows, :], x_ref.at[rows, :], sems.at[r])

    def w_copy(t):
        cols = pl.ds(t * D, D)
        return pltpu.make_async_copy(wqkv_hbm.at[:, cols], wqkv_ref.at[:, cols], sems.at[NR + t])

    late = ((wg_hbm, wg_ref), (wu_hbm, wu_ref), (wd_hbm, wd_ref), (wo_hbm, wo_ref))

    def late_copy(t):
        return pltpu.make_async_copy(late[t][0], late[t][1], sems.at[NR + 3 + t])

    def o_copy(j, row0):
        dst = pl.ds(pl.multiple_of(row0 + j * TO, TO), TO)
        return pltpu.make_async_copy(o_scr.at[pl.ds(j * TO, TO), :], o_hbm.at[dst, :], osems.at[j])

    @pl.when(step == 0)
    def _():
        x_copy(0).start()
        x_copy(1).start()
        w_copy(1).start()
        m_scr[16:40, :] = jnp.zeros((24, TQ), F32)
        m_scr[40:48, :] = jnp.full((8, TQ), -jnp.inf, F32)
        y_scr[...] = jnp.zeros((TQ, D), F32)

        upper = lax.broadcasted_iota(jnp.int32, (TR, 128), 1) >= 64
        low4 = lax.broadcasted_iota(jnp.int32, (8, TR), 0) < 4

        def row0(r):
            return r * TR if isinstance(r, int) else pl.multiple_of(r * TR, TR)

        def layernorm(r):
            rows = pl.ds(row0(r), TR)
            x = x_ref[rows, :].astype(F32)
            mu = jnp.mean(x, axis=-1, keepdims=True)
            xc = x - mu
            var = jnp.mean(xc * xc, axis=-1, keepdims=True)
            xn_scr[rows, :] = (xc * lax.rsqrt(var + EPS)).astype(BF16)

        def v_part(r):
            rows = pl.ds(row0(r), TR)
            vt = jnp.dot(xn_scr[rows, :], wqkv_ref[:, 2 * D:3 * D], preferred_element_type=F32).T
            for p in range(H // 2):
                mid = vt[40 * p + 16:40 * p + 24, :]
                vt_scr[48 * p:48 * p + 16, rows] = vt[40 * p:40 * p + 16, :]
                vt_scr[48 * p + 16:48 * p + 24, rows] = jnp.where(low4, mid, 1.0)
                vt_scr[48 * p + 24:48 * p + 32, rows] = jnp.where(low4, 1.0, mid)
                vt_scr[48 * p + 32:48 * p + 48, rows] = vt[40 * p + 24:40 * p + 40, :]

        def qk_part(r, t):
            rows = pl.ds(row0(r), TR)
            dst = (q_scr, k_scr)[t]
            y = jnp.dot(xn_scr[rows, :], wqkv_ref[:, t * D:(t + 1) * D], preferred_element_type=F32)
            if t == 0:
                y = y * QSCALE
            gs = [y[:, g * 128:(g + 1) * 128] for g in range(NG)]
            for g in range(NG):
                dst[g, rows, :] = gs[g].astype(BF16)
            for g in range(NG - 1):
                dst[NG + g, rows, :] = jnp.where(upper, gs[g], gs[g + 1]).astype(BF16)
            if t == 0:
                yt = y.astype(BF16).astype(F32).T
                qtile = r // (TQ // TR)
                cols = pl.ds(row0(r % (TQ // TR)), TR)
                for p in range(H // 2):
                    qt_scr[p * NQ + qtile, :, cols] = yt[40 * p:40 * p + 40, :]
            else:
                ka = y[TK - 2 * NV:TK - NV, :].astype(BF16).astype(F32)
                kc = y[TK - NV:TK, :].astype(BF16).astype(F32)
                kw_scr[r] = (pltpu.bitcast(ka, U32) & U32(0xFFFF0000)) | (pltpu.bitcast(kc, U32) >> 16)

        def kb_part(r, j0=0, j1=D):
            w = kw_scr[r]
            for j in range(j0, j1):
                bc = jnp.broadcast_to(w[:, j:j + 1], (NV, 128))
                kb_scr[2 * r, j * NV:(j + 1) * NV, :] = pltpu.bitcast(bc & U32(0xFFFF0000), F32)
                kb_scr[2 * r + 1, j * NV:(j + 1) * NV, :] = pltpu.bitcast(bc << 16, F32)

        x_copy(0).wait()
        w_copy(2).start()
        x_copy(2).start()
        w_copy(0).start()
        layernorm(0)
        x_copy(1).wait()
        layernorm(1)
        w_copy(1).wait()
        qk_part(0, 1)
        qk_part(1, 1)
        w_copy(2).wait()
        x_copy(2).wait()
        for r in range(3, NR):
            x_copy(r).start()
        layernorm(2)
        v_part(0)
        w_copy(0).wait()
        for t in range(4):
            late_copy(t).start()

        def rows_body(r, carry):
            @pl.when(r + 3 < NR)
            def _():
                x_copy(r + 3).wait()
            kb_part(r, 0, 214)
            qk_part(r, 0)
            kb_part(r, 214, 427)
            v_part(r + 1)
            kb_part(r, 427, D)
            qk_part(r + 2, 1)
            layernorm(jnp.where(r + 3 < NR, r + 3, 0))
            return carry

        lax.fori_loop(0, NR - 2, rows_body, 0)
        kb_part(NR - 2)
        qk_part(NR - 2, 0)
        kb_part(NR - 1)
        v_part(NR - 1)
        qk_part(NR - 1, 0)

        gx, qm = item_q(0, 0)
        mrun = None
        for c in range(NCS + LEAD):
            if c == NCS:
                m_scr[0:8, :] = jnp.broadcast_to(jnp.max(mrun, axis=0, keepdims=True), (8, TQ))
                mrun = None
            mrun = stage1_chunk(c // NCS, gx, qm, c, mrun, (0, 0, 0))
        m_scr[8:16, :] = mrun
        for t in range(4):
            late_copy(t).wait()

    q0 = pl.multiple_of(step * TQ, TQ)
    low4q = lax.broadcasted_iota(jnp.int32, (8, TQ), 0) < 4

    def finish_pair(p, acc_e, acc_o):
        inv_e = 1.0 / acc_e[20:21, :]
        inv_o = 1.0 / acc_o[0:1, :]
        r0 = pl.multiple_of(p * 40, 8)
        ot_scr[pl.ds(r0, 16), :] = acc_e[0:16, :] * inv_e
        ot_scr[pl.ds(r0 + 16, 8), :] = jnp.where(low4q, acc_e[16:24, :] * inv_e, acc_o[0:8, :] * inv_o)
        ot_scr[pl.ds(r0 + 24, 16), :] = acc_o[8:24, :] * inv_o

    def body(it, carry):
        m, mrun = carry
        h0 = it * HPI
        wrap = h0 + HPI >= H
        tn = jnp.where(wrap, jnp.minimum(step + 1, NQ - 1), step)
        hn = jnp.where(wrap, 0, h0 + HPI)
        fcols = pl.ds(pl.multiple_of(it * FL, FL), FL)

        def ffn_up():
            xn = xn_scr[pl.ds(q0, TQ), :]
            g = jnp.dot(xn, wg_ref[:, fcols], preferred_element_type=F32)
            u = jnp.dot(xn, wu_ref[:, fcols], preferred_element_type=F32)
            return (g * jax.nn.sigmoid(g) * u).astype(BF16)

        def ffn_down(hidden):
            part = jnp.dot(hidden, wd_ref[fcols, :], preferred_element_type=F32)
            prev = jnp.where(it == 0, x_ref[pl.ds(q0, TQ), :].astype(F32), y_scr[...])
            y_scr[...] = prev + part

        m_next = None
        accs = []
        parts = []
        acc = None
        cur = None
        for t in range(HPI * NCK):
            if t == 0:
                hidden = ffn_up()
            elif t == 1:
                ffn_down(hidden)
            u = t + NCS + LEAD
            i1, c1 = divmod(u, NCK)
            if cur is None or c1 == 0:
                if i1 < HPI:
                    cur = item_q(h0 + i1, q0)
                    vinfo = (h0 + i1, i1 % 2, step)
                else:
                    cur = item_q(hn + (i1 - HPI), pl.multiple_of(tn * TQ, TQ))
                    vinfo = (hn + (i1 - HPI), i1 % 2, tn)
            if u % NCS == 0:
                mrun = None
            mrun = stage1_chunk(u // NCS, cur[0], cur[1], c1, mrun, vinfo)
            if u % NCS == NCS - 1:
                m_next = jnp.max(mrun, axis=0, keepdims=True)
            i2, c2 = divmod(t, NCK)
            acc = stage2_chunk(t // NCS, h0 + i2, m, c2, m_scr[16:40, :] if t % NCS == 0 else acc)
            if t % NCS == NCS - 1:
                parts.append((m, acc))
                m = m_next
            if c2 == NCK - 1:
                mt = parts[0][0]
                for pm, _ in parts[1:]:
                    mt = jnp.maximum(mt, pm)
                tot = None
                for pm, pa in parts:
                    term = pa * jnp.exp2(pm - mt)
                    tot = term if tot is None else tot + term
                parts = []
                accs.append(tot)
                if i2 % 2 == 1:
                    finish_pair((h0 + i2) // 2, accs[-2], accs[-1])
        return m, mrun

    m_fin, mrun_fin = lax.fori_loop(0, H // HPI, body, (m_scr[0:1, :], m_scr[8:16, :]))
    m_scr[0:8, :] = jnp.broadcast_to(m_fin, (8, TQ))
    m_scr[8:16, :] = mrun_fin

    @pl.when(step > 0)
    def _():
        for j in range(TQ // TO):
            o_copy(j, q0 - TQ).wait()

    f0 = FL * (H // HPI)
    xn = xn_scr[pl.ds(q0, TQ), :]
    g = jnp.dot(xn, wg_ref[:, f0:F], preferred_element_type=F32)
    u = jnp.dot(xn, wu_ref[:, f0:F], preferred_element_type=F32)
    hid = (g * jax.nn.sigmoid(g) * u).astype(BF16)
    for j in range(TQ // TO):
        o = ot_scr[:, j * TO:(j + 1) * TO].T.astype(BF16)
        attn = jnp.dot(o, wo_ref[...], preferred_element_type=F32)
        attn = attn + jnp.dot(hid[j * TO:(j + 1) * TO, :], wd_ref[f0:F, :], preferred_element_type=F32)
        o_scr[j * TO:(j + 1) * TO, :] = (y_scr[j * TO:(j + 1) * TO, :] + attn).astype(BF16)
        o_copy(j, q0).start()

    @pl.when(step == NQ - 1)
    def _():
        for j in range(TQ // TO):
            o_copy(j, q0).wait()


@jax.jit
def pallas_parallel_sum__mha_block__swiglu_ffn__prompt_kernel(
    A_x: jax.Array,
    A_wqkv: jax.Array,
    A_wo: jax.Array,
    B_x: jax.Array,
    B_w_gate: jax.Array,
    B_w_up: jax.Array,
    B_w_down: jax.Array,
):
    del B_x
    x = A_x.reshape(S, D)
    hbm = pl.BlockSpec(memory_space=pl.ANY)
    out = pl.pallas_call(
        _kernel,
        grid=(NQ,),
        in_specs=[hbm] * 6,
        out_specs=hbm,
        out_shape=jax.ShapeDtypeStruct((S, D), A_x.dtype),
        scratch_shapes=[
            pltpu.VMEM((S, D), BF16),
            pltpu.VMEM((D, 3 * D), BF16),
            pltpu.VMEM((D, D), BF16),
            pltpu.VMEM((D, F), BF16),
            pltpu.VMEM((D, F), BF16),
            pltpu.VMEM((F, D), BF16),
            pltpu.SemaphoreType.DMA((NR + 7,)),
            pltpu.VMEM((S, D), BF16),
            pltpu.VMEM((NGX, S, 128), BF16),
            pltpu.VMEM((NGX, S, 128), BF16),
            pltpu.VMEM((H * 24, S), F32),
            pltpu.VMEM((2, S // NSP, TQ), F32),
            pltpu.VMEM((D, TQ), F32),
            pltpu.VMEM((48, TQ), F32),
            pltpu.VMEM((TQ, D), F32),
            pltpu.VMEM((TQ, D), BF16),
            pltpu.SemaphoreType.DMA((TQ // TO,)),
            pltpu.VMEM((H // 2 * NQ, 2 * DH, TQ), F32),
            pltpu.VMEM((NCK, D * NV, 128), F32),
            pltpu.VMEM((NR, NV, D), U32),
        ],
        compiler_params=pltpu.CompilerParams(
            dimension_semantics=("arbitrary",),
            vmem_limit_bytes=112 * 1024 * 1024,
        ),
    )(x, A_wqkv, A_wo, B_w_gate, B_w_up, B_w_down)
    return out.reshape(1, S, D)
```

```python
import math

import jax
import jax.numpy as jnp
from jax import lax
import jax.experimental.pallas as pl
import jax.experimental.pallas.tpu as pltpu

S, D, H, DH, F = 2048, 640, 32, 20, 1536
TQ = 512
TK = 128
NV = 8
TR = 256
TO = 128
HPI = 8
NSP = 4
LEAD = 1
FL = 128
NCH = 2
NG = D // 128
NGX = 2 * NG - 1
NQ = S // TQ
NR = S // TR
NCK = S // TK
NCS = NCK // NSP
EPS = 1e-5
QSCALE = (DH ** -0.5) * math.log2(math.e)
NT = (((1,), (1,)), ((), ()))
F32 = jnp.float32
BF16 = jnp.bfloat16
U32 = jnp.uint32


def _kernel(x_hbm, wqkv_hbm, wo_hbm, wg_hbm, wu_hbm, wd_hbm, o_hbm,
            x_ref, wqkv_ref, wo_ref, wg_ref, wu_ref, wd_ref, sems,
            xn_scr, q_scr, k_scr, vt_scr, s2_scr, ot_scr, m_scr, y_scr, o_scr, osems,
            qt_scr, kb_scr, kw_scr):
    step = pl.program_id(0)
    lane_q = lax.broadcasted_iota(jnp.int32, (TQ, 128), 1)

    def item_q(h, qrow):
        a = h * DH
        g = a // 128
        lo = a % 128
        gx = jnp.where(lo > 128 - DH, g + NG, g)
        rel = (lane_q - lo) & 127
        q = q_scr[gx, pl.ds(qrow, TQ), :]
        return gx, jnp.where(rel < DH, q.astype(F32), 0.0).astype(BF16)

    def vpu_scores(h, parity, qtile, c):
        ncc = TQ // 128
        qi = (h // 2) * NQ + qtile
        kr = pl.multiple_of(h * (DH * NV), NV)
        accs = [None] * NCH
        for d in range(DH):
            row = parity * DH + d
            qb = jnp.concatenate(
                [jnp.broadcast_to(qt_scr[qi, row:row + 1, cc * 128:(cc + 1) * 128], (NV, 128))
                 for cc in range(ncc)], axis=1)
            kb = kb_scr[c, pl.ds(kr + d * NV, NV), :]
            t = jnp.concatenate([kb] * ncc, axis=1) * qb
            j = d % NCH
            accs[j] = t if accs[j] is None else accs[j] + t
        acc = accs[0]
        for a in accs[1:]:
            acc = acc + a
        return acc

    def stage1_chunk(part, gx, qm, c, mrun, vinfo):
        r0 = (c % NCS) * TK
        nm = TK - 2 * NV if c % 2 == 0 else TK
        if mrun is None:
            mrun = m_scr[40:48, :]
        v = vpu_scores(*vinfo, c)
        rv = ((c % NCS) // 2 * 2 + 1) * TK - 2 * NV + (c % 2) * NV
        s2_scr[part % 2, rv:rv + NV, :] = v
        s = lax.dot_general(k_scr[gx, c * TK:c * TK + nm, :], qm, NT, preferred_element_type=F32)
        s2_scr[part % 2, r0:r0 + nm, :] = s
        mrun = jnp.maximum(mrun, v)
        return jnp.maximum(mrun, jnp.max(s.reshape(nm // 8, 8, TQ), axis=0))

    def stage2_chunk(part, h, m, c, acc):
        r0 = (c % NCS) * TK
        p = jnp.exp2(s2_scr[part % 2, r0:r0 + TK, :] - m).astype(BF16)
        vt = vt_scr[pl.ds(pl.multiple_of(h * 24, 8), 24), c * TK:(c + 1) * TK]
        return acc + jnp.dot(vt, p, preferred_element_type=F32)

    def x_copy(r):
        rows = pl.ds(pl.multiple_of(r * TR, TR), TR)
        return pltpu.make_async_copy(x_hbm.at[rows, :], x_ref.at[rows, :], sems.at[r])

    def w_copy(t):
        cols = pl.ds(t * D, D)
        return pltpu.make_async_copy(wqkv_hbm.at[:, cols], wqkv_ref.at[:, cols], sems.at[NR + t])

    late = ((wg_hbm, wg_ref), (wu_hbm, wu_ref), (wd_hbm, wd_ref), (wo_hbm, wo_ref))

    def late_copy(t):
        return pltpu.make_async_copy(late[t][0], late[t][1], sems.at[NR + 3 + t])

    def o_copy(j, row0):
        dst = pl.ds(pl.multiple_of(row0 + j * TO, TO), TO)
        return pltpu.make_async_copy(o_scr.at[pl.ds(j * TO, TO), :], o_hbm.at[dst, :], osems.at[j])

    @pl.when(step == 0)
    def _():
        x_copy(0).start()
        x_copy(1).start()
        w_copy(1).start()
        m_scr[16:40, :] = jnp.zeros((24, TQ), F32)
        m_scr[40:48, :] = jnp.full((8, TQ), -jnp.inf, F32)
        y_scr[...] = jnp.zeros((TQ, D), F32)

        upper = lax.broadcasted_iota(jnp.int32, (TR, 128), 1) >= 64
        low4 = lax.broadcasted_iota(jnp.int32, (8, TR), 0) < 4

        def row0(r):
            return r * TR if isinstance(r, int) else pl.multiple_of(r * TR, TR)

        def layernorm(r):
            rows = pl.ds(row0(r), TR)
            x = x_ref[rows, :].astype(F32)
            mu = jnp.mean(x, axis=-1, keepdims=True)
            xc = x - mu
            var = jnp.mean(xc * xc, axis=-1, keepdims=True)
            xn_scr[rows, :] = (xc * lax.rsqrt(var + EPS)).astype(BF16)

        def v_part(r):
            rows = pl.ds(row0(r), TR)
            vt = jnp.dot(xn_scr[rows, :], wqkv_ref[:, 2 * D:3 * D], preferred_element_type=F32).T
            for p in range(H // 2):
                mid = vt[40 * p + 16:40 * p + 24, :]
                vt_scr[48 * p:48 * p + 16, rows] = vt[40 * p:40 * p + 16, :]
                vt_scr[48 * p + 16:48 * p + 24, rows] = jnp.where(low4, mid, 1.0)
                vt_scr[48 * p + 24:48 * p + 32, rows] = jnp.where(low4, 1.0, mid)
                vt_scr[48 * p + 32:48 * p + 48, rows] = vt[40 * p + 24:40 * p + 40, :]

        def qk_part(r, t):
            rows = pl.ds(row0(r), TR)
            dst = (q_scr, k_scr)[t]
            y = jnp.dot(xn_scr[rows, :], wqkv_ref[:, t * D:(t + 1) * D], preferred_element_type=F32)
            if t == 0:
                y = y * QSCALE
            gs = [y[:, g * 128:(g + 1) * 128] for g in range(NG)]
            for g in range(NG):
                dst[g, rows, :] = gs[g].astype(BF16)
            for g in range(NG - 1):
                dst[NG + g, rows, :] = jnp.where(upper, gs[g], gs[g + 1]).astype(BF16)
            if t == 0:
                yt = y.astype(BF16).astype(F32).T
                qtile = r // (TQ // TR)
                cols = pl.ds(row0(r % (TQ // TR)), TR)
                for p in range(H // 2):
                    qt_scr[p * NQ + qtile, :, cols] = yt[40 * p:40 * p + 40, :]
            else:
                ka = y[TK - 2 * NV:TK - NV, :].astype(BF16).astype(F32)
                kc = y[TK - NV:TK, :].astype(BF16).astype(F32)
                kw_scr[r] = (pltpu.bitcast(ka, U32) & U32(0xFFFF0000)) | (pltpu.bitcast(kc, U32) >> 16)

        def kb_part(r, j0=0, j1=D):
            w = kw_scr[r]
            for j in range(j0, j1):
                bc = jnp.broadcast_to(w[:, j:j + 1], (NV, 128))
                kb_scr[2 * r, j * NV:(j + 1) * NV, :] = pltpu.bitcast(bc & U32(0xFFFF0000), F32)
                kb_scr[2 * r + 1, j * NV:(j + 1) * NV, :] = pltpu.bitcast(bc << 16, F32)

        x_copy(0).wait()
        w_copy(2).start()
        x_copy(2).start()
        w_copy(0).start()
        layernorm(0)
        x_copy(1).wait()
        layernorm(1)
        w_copy(1).wait()
        qk_part(0, 1)
        qk_part(1, 1)
        w_copy(2).wait()
        x_copy(2).wait()
        for r in range(3, NR):
            x_copy(r).start()
        layernorm(2)
        v_part(0)
        w_copy(0).wait()
        for t in range(4):
            late_copy(t).start()

        def rows_body(r, carry):
            @pl.when(r + 3 < NR)
            def _():
                x_copy(r + 3).wait()
            kb_part(r, 0, 214)
            qk_part(r, 0)
            kb_part(r, 214, 427)
            v_part(r + 1)
            kb_part(r, 427, D)
            qk_part(r + 2, 1)
            layernorm(jnp.where(r + 3 < NR, r + 3, 0))
            return carry

        lax.fori_loop(0, NR - 2, rows_body, 0)
        kb_part(NR - 2)
        qk_part(NR - 2, 0)
        kb_part(NR - 1)
        v_part(NR - 1)
        qk_part(NR - 1, 0)

        gx, qm = item_q(0, 0)
        mrun = None
        for c in range(NCS + LEAD):
            if c == NCS:
                m_scr[0:8, :] = jnp.broadcast_to(jnp.max(mrun, axis=0, keepdims=True), (8, TQ))
                mrun = None
            mrun = stage1_chunk(c // NCS, gx, qm, c, mrun, (0, 0, 0))
        m_scr[8:16, :] = mrun
        for t in range(4):
            late_copy(t).wait()

    q0 = pl.multiple_of(step * TQ, TQ)
    low4q = lax.broadcasted_iota(jnp.int32, (8, TQ), 0) < 4

    def finish_pair(p, acc_e, acc_o):
        inv_e = 1.0 / acc_e[20:21, :]
        inv_o = 1.0 / acc_o[0:1, :]
        r0 = pl.multiple_of(p * 40, 8)
        ot_scr[pl.ds(r0, 16), :] = acc_e[0:16, :] * inv_e
        ot_scr[pl.ds(r0 + 16, 8), :] = jnp.where(low4q, acc_e[16:24, :] * inv_e, acc_o[0:8, :] * inv_o)
        ot_scr[pl.ds(r0 + 24, 16), :] = acc_o[8:24, :] * inv_o

    def body(it, carry):
        m, mrun = carry
        h0 = it * HPI
        wrap = h0 + HPI >= H
        tn = jnp.where(wrap, jnp.minimum(step + 1, NQ - 1), step)
        hn = jnp.where(wrap, 0, h0 + HPI)
        fcols = pl.ds(pl.multiple_of(it * FL, FL), FL)

        def ffn_up():
            xn = xn_scr[pl.ds(q0, TQ), :]
            g = jnp.dot(xn, wg_ref[:, fcols], preferred_element_type=F32)
            u = jnp.dot(xn, wu_ref[:, fcols], preferred_element_type=F32)
            return (g * jax.nn.sigmoid(g) * u).astype(BF16)

        def ffn_down(hidden):
            part = jnp.dot(hidden, wd_ref[fcols, :], preferred_element_type=F32)
            prev = jnp.where(it == 0, x_ref[pl.ds(q0, TQ), :].astype(F32), y_scr[...])
            y_scr[...] = prev + part

        m_next = m
        accs = []
        parts = []
        acc = None
        cur = None
        for t in range(HPI * NCK):
            if t == 0:
                hidden = ffn_up()
            elif t == 1:
                ffn_down(hidden)
            u = t + NCS + LEAD
            i1, c1 = divmod(u, NCK)
            if cur is None or c1 == 0:
                if i1 < HPI:
                    cur = item_q(h0 + i1, q0)
                    vinfo = (h0 + i1, i1 % 2, step)
                else:
                    cur = item_q(hn + (i1 - HPI), pl.multiple_of(tn * TQ, TQ))
                    vinfo = (hn + (i1 - HPI), i1 % 2, tn)
            if u % NCS == 0:
                mrun = None
            mrun = stage1_chunk(u // NCS, cur[0], cur[1], c1, mrun, vinfo)
            if u % NCS == NCS - 1:
                m_range = jnp.max(mrun, axis=0, keepdims=True)
                m_next = m_range if c1 < NCS else jnp.maximum(m_next, m_range)
            i2, c2 = divmod(t, NCK)
            acc = stage2_chunk(t // NCS, h0 + i2, m, c2, m_scr[16:40, :] if t % NCS == 0 else acc)
            if t % NCS == NCS - 1:
                parts.append((m, acc))
                m = m_next
            if c2 == NCK - 1:
                mt, tot = parts[-1]
                for pm, pa in parts[:-1]:
                    tot = tot + pa * jnp.exp2(pm - mt)
                parts = []
                accs.append(tot)
                if i2 % 2 == 1:
                    finish_pair((h0 + i2) // 2, accs[-2], accs[-1])
        return m, mrun

    m_fin, mrun_fin = lax.fori_loop(0, H // HPI, body, (m_scr[0:1, :], m_scr[8:16, :]))
    m_scr[0:8, :] = jnp.broadcast_to(m_fin, (8, TQ))
    m_scr[8:16, :] = mrun_fin

    @pl.when(step > 0)
    def _():
        for j in range(TQ // TO):
            o_copy(j, q0 - TQ).wait()

    f0 = FL * (H // HPI)
    xn = xn_scr[pl.ds(q0, TQ), :]
    g = jnp.dot(xn, wg_ref[:, f0:F], preferred_element_type=F32)
    u = jnp.dot(xn, wu_ref[:, f0:F], preferred_element_type=F32)
    hid = (g * jax.nn.sigmoid(g) * u).astype(BF16)
    for j in range(TQ // TO):
        o = ot_scr[:, j * TO:(j + 1) * TO].T.astype(BF16)
        attn = jnp.dot(o, wo_ref[...], preferred_element_type=F32)
        attn = attn + jnp.dot(hid[j * TO:(j + 1) * TO, :], wd_ref[f0:F, :], preferred_element_type=F32)
        o_scr[j * TO:(j + 1) * TO, :] = (y_scr[j * TO:(j + 1) * TO, :] + attn).astype(BF16)
        o_copy(j, q0).start()

    @pl.when(step == NQ - 1)
    def _():
        for j in range(TQ // TO):
            o_copy(j, q0).wait()


@jax.jit
def pallas_parallel_sum__mha_block__swiglu_ffn__prompt_kernel(
    A_x: jax.Array,
    A_wqkv: jax.Array,
    A_wo: jax.Array,
    B_x: jax.Array,
    B_w_gate: jax.Array,
    B_w_up: jax.Array,
    B_w_down: jax.Array,
):
    del B_x
    x = A_x.reshape(S, D)
    hbm = pl.BlockSpec(memory_space=pl.ANY)
    out = pl.pallas_call(
        _kernel,
        grid=(NQ,),
        in_specs=[hbm] * 6,
        out_specs=hbm,
        out_shape=jax.ShapeDtypeStruct((S, D), A_x.dtype),
        scratch_shapes=[
            pltpu.VMEM((S, D), BF16),
            pltpu.VMEM((D, 3 * D), BF16),
            pltpu.VMEM((D, D), BF16),
            pltpu.VMEM((D, F), BF16),
            pltpu.VMEM((D, F), BF16),
            pltpu.VMEM((F, D), BF16),
            pltpu.SemaphoreType.DMA((NR + 7,)),
            pltpu.VMEM((S, D), BF16),
            pltpu.VMEM((NGX, S, 128), BF16),
            pltpu.VMEM((NGX, S, 128), BF16),
            pltpu.VMEM((H * 24, S), F32),
            pltpu.VMEM((2, S // NSP, TQ), F32),
            pltpu.VMEM((D, TQ), F32),
            pltpu.VMEM((48, TQ), F32),
            pltpu.VMEM((TQ, D), F32),
            pltpu.VMEM((TQ, D), BF16),
            pltpu.SemaphoreType.DMA((TQ // TO,)),
            pltpu.VMEM((H // 2 * NQ, 2 * DH, TQ), F32),
            pltpu.VMEM((NCK, D * NV, 128), F32),
            pltpu.VMEM((NR, NV, D), U32),
        ],
        compiler_params=pltpu.CompilerParams(
            dimension_semantics=("arbitrary",),
            vmem_limit_bytes=112 * 1024 * 1024,
        ),
    )(x, A_wqkv, A_wo, B_w_gate, B_w_up, B_w_down)
    return out.reshape(1, S, D)
```

```python
import math

import jax
import jax.numpy as jnp
from jax import lax
import jax.experimental.pallas as pl
import jax.experimental.pallas.tpu as pltpu

S, D, H, DH, F = 2048, 640, 32, 20, 1536
TQ = 512
TK = 128
NV = 8
TR = 256
TO = 128
HPI = 8
NSP = 4
LEAD = 1
FL = 128
NCH = 2
NG = D // 128
NGX = 2 * NG - 1
NQ = S // TQ
NR = S // TR
NCK = S // TK
NCS = NCK // NSP
EPS = 1e-5
QSCALE = (DH ** -0.5) * math.log2(math.e)
NT = (((1,), (1,)), ((), ()))
F32 = jnp.float32
BF16 = jnp.bfloat16
U32 = jnp.uint32


def _kernel(x_hbm, wqkv_hbm, wo_hbm, wg_hbm, wu_hbm, wd_hbm, o_hbm,
            x_ref, wqkv_ref, wo_ref, wg_ref, wu_ref, wd_ref, sems,
            xn_scr, q_scr, k_scr, vt_scr, s2_scr, ot_scr, m_scr, y_scr, o_scr, osems,
            qt_scr, kb_scr, kw_scr):
    step = pl.program_id(0)
    lane_q = lax.broadcasted_iota(jnp.int32, (TQ, 128), 1)

    def item_q(h, qrow):
        a = h * DH
        g = a // 128
        lo = a % 128
        gx = jnp.where(lo > 128 - DH, g + NG, g)
        rel = (lane_q - lo) & 127
        q = q_scr[gx, pl.ds(qrow, TQ), :]
        return gx, jnp.where(rel < DH, q.astype(F32), 0.0).astype(BF16)

    def q_rows(h, parity, qtile):
        qi = (h // 2) * NQ + qtile
        return [jnp.concatenate(
            [jnp.broadcast_to(qt_scr[qi, row:row + 1, cc * 128:(cc + 1) * 128], (NV, 128))
             for cc in range(TQ // 128)], axis=1) for row in range(parity * DH, parity * DH + DH)]

    def vpu_scores(h, qbs, c):
        kb = kb_scr[c, pl.ds(pl.multiple_of(h * (DH * NV), NV), DH * NV), :]
        kb = jnp.concatenate([kb] * (TQ // 128), axis=1)
        accs = [None] * NCH
        for d in range(DH):
            t = kb[d * NV:(d + 1) * NV, :] * qbs[d]
            j = d % NCH
            accs[j] = t if accs[j] is None else accs[j] + t
        acc = accs[0]
        for a in accs[1:]:
            acc = acc + a
        return acc

    def stage1_chunk(part, gx, qm, c, mrun, vinfo):
        r0 = (c % NCS) * TK
        nm = TK - 2 * NV if c % 2 == 0 else TK
        if mrun is None:
            mrun = m_scr[40:48, :]
        v = vpu_scores(*vinfo, c)
        rv = ((c % NCS) // 2 * 2 + 1) * TK - 2 * NV + (c % 2) * NV
        s2_scr[part % 2, rv:rv + NV, :] = v
        s = lax.dot_general(k_scr[gx, c * TK:c * TK + nm, :], qm, NT, preferred_element_type=F32)
        s2_scr[part % 2, r0:r0 + nm, :] = s
        mrun = jnp.maximum(mrun, v)
        return jnp.maximum(mrun, jnp.max(s.reshape(nm // 8, 8, TQ), axis=0))

    def stage2_chunk(part, h, m, c, acc):
        r0 = (c % NCS) * TK
        p = jnp.exp2(s2_scr[part % 2, r0:r0 + TK, :] - m).astype(BF16)
        vt = vt_scr[pl.ds(pl.multiple_of(h * 24, 8), 24), c * TK:(c + 1) * TK]
        return acc + jnp.dot(vt, p, preferred_element_type=F32)

    def x_copy(r):
        rows = pl.ds(pl.multiple_of(r * TR, TR), TR)
        return pltpu.make_async_copy(x_hbm.at[rows, :], x_ref.at[rows, :], sems.at[r])

    def w_copy(t):
        cols = pl.ds(t * D, D)
        return pltpu.make_async_copy(wqkv_hbm.at[:, cols], wqkv_ref.at[:, cols], sems.at[NR + t])

    late = ((wg_hbm, wg_ref), (wu_hbm, wu_ref), (wd_hbm, wd_ref), (wo_hbm, wo_ref))

    def late_copy(t):
        return pltpu.make_async_copy(late[t][0], late[t][1], sems.at[NR + 3 + t])

    def o_copy(j, row0):
        dst = pl.ds(pl.multiple_of(row0 + j * TO, TO), TO)
        return pltpu.make_async_copy(o_scr.at[pl.ds(j * TO, TO), :], o_hbm.at[dst, :], osems.at[j])

    @pl.when(step == 0)
    def _():
        x_copy(0).start()
        x_copy(1).start()
        w_copy(1).start()
        m_scr[16:40, :] = jnp.zeros((24, TQ), F32)
        m_scr[40:48, :] = jnp.full((8, TQ), -jnp.inf, F32)
        y_scr[...] = jnp.zeros((TQ, D), F32)

        upper = lax.broadcasted_iota(jnp.int32, (TR, 128), 1) >= 64
        low4 = lax.broadcasted_iota(jnp.int32, (8, TR), 0) < 4

        def row0(r):
            return r * TR if isinstance(r, int) else pl.multiple_of(r * TR, TR)

        def layernorm(r):
            rows = pl.ds(row0(r), TR)
            x = x_ref[rows, :].astype(F32)
            mu = jnp.mean(x, axis=-1, keepdims=True)
            xc = x - mu
            var = jnp.mean(xc * xc, axis=-1, keepdims=True)
            xn_scr[rows, :] = (xc * lax.rsqrt(var + EPS)).astype(BF16)

        def v_part(r):
            rows = pl.ds(row0(r), TR)
            vt = jnp.dot(xn_scr[rows, :], wqkv_ref[:, 2 * D:3 * D], preferred_element_type=F32).T
            for p in range(H // 2):
                mid = vt[40 * p + 16:40 * p + 24, :]
                vt_scr[48 * p:48 * p + 16, rows] = vt[40 * p:40 * p + 16, :]
                vt_scr[48 * p + 16:48 * p + 24, rows] = jnp.where(low4, mid, 1.0)
                vt_scr[48 * p + 24:48 * p + 32, rows] = jnp.where(low4, 1.0, mid)
                vt_scr[48 * p + 32:48 * p + 48, rows] = vt[40 * p + 24:40 * p + 40, :]

        def qk_part(r, t):
            rows = pl.ds(row0(r), TR)
            dst = (q_scr, k_scr)[t]
            y = jnp.dot(xn_scr[rows, :], wqkv_ref[:, t * D:(t + 1) * D], preferred_element_type=F32)
            if t == 0:
                y = y * QSCALE
            gs = [y[:, g * 128:(g + 1) * 128] for g in range(NG)]
            for g in range(NG):
                dst[g, rows, :] = gs[g].astype(BF16)
            for g in range(NG - 1):
                dst[NG + g, rows, :] = jnp.where(upper, gs[g], gs[g + 1]).astype(BF16)
            if t == 0:
                yt = y.astype(BF16).astype(F32).T
                qtile = r // (TQ // TR)
                cols = pl.ds(row0(r % (TQ // TR)), TR)
                for p in range(H // 2):
                    qt_scr[p * NQ + qtile, :, cols] = yt[40 * p:40 * p + 40, :]
            else:
                ka = y[TK - 2 * NV:TK - NV, :].astype(BF16).astype(F32)
                kc = y[TK - NV:TK, :].astype(BF16).astype(F32)
                kw_scr[r] = (pltpu.bitcast(ka, U32) & U32(0xFFFF0000)) | (pltpu.bitcast(kc, U32) >> 16)

        def kb_part(r, j0=0, j1=D):
            w = kw_scr[r]
            bc = jnp.concatenate(
                [jnp.broadcast_to(w[:, j:j + 1], (NV, 128)) for j in range(j0, j1)], axis=0)
            kb_scr[2 * r, j0 * NV:j1 * NV, :] = pltpu.bitcast(bc & U32(0xFFFF0000), F32)
            kb_scr[2 * r + 1, j0 * NV:j1 * NV, :] = pltpu.bitcast(bc << 16, F32)

        x_copy(0).wait()
        w_copy(2).start()
        x_copy(2).start()
        w_copy(0).start()
        layernorm(0)
        x_copy(1).wait()
        layernorm(1)
        w_copy(1).wait()
        qk_part(0, 1)
        qk_part(1, 1)
        w_copy(2).wait()
        x_copy(2).wait()
        for r in range(3, NR):
            x_copy(r).start()
        layernorm(2)
        v_part(0)
        w_copy(0).wait()
        for t in range(4):
            late_copy(t).start()

        def rows_body(r, carry):
            @pl.when(r + 3 < NR)
            def _():
                x_copy(r + 3).wait()
            kb_part(r, 0, 214)
            qk_part(r, 0)
            kb_part(r, 214, 427)
            v_part(r + 1)
            kb_part(r, 427, D)
            qk_part(r + 2, 1)
            layernorm(jnp.where(r + 3 < NR, r + 3, 0))
            return carry

        lax.fori_loop(0, NR - 2, rows_body, 0)
        kb_part(NR - 2)
        qk_part(NR - 2, 0)
        kb_part(NR - 1)
        v_part(NR - 1)
        qk_part(NR - 1, 0)

        gx, qm = item_q(0, 0)
        vinfo = (0, q_rows(0, 0, 0))
        mrun = None
        for c in range(NCS + LEAD):
            if c == NCS:
                m_scr[0:8, :] = jnp.broadcast_to(jnp.max(mrun, axis=0, keepdims=True), (8, TQ))
                mrun = None
            mrun = stage1_chunk(c // NCS, gx, qm, c, mrun, vinfo)
        m_scr[8:16, :] = mrun
        for t in range(4):
            late_copy(t).wait()

    q0 = pl.multiple_of(step * TQ, TQ)
    low4q = lax.broadcasted_iota(jnp.int32, (8, TQ), 0) < 4

    def finish_pair(p, acc_e, acc_o):
        inv_e = 1.0 / acc_e[20:21, :]
        inv_o = 1.0 / acc_o[0:1, :]
        r0 = pl.multiple_of(p * 40, 8)
        ot_scr[pl.ds(r0, 16), :] = acc_e[0:16, :] * inv_e
        ot_scr[pl.ds(r0 + 16, 8), :] = jnp.where(low4q, acc_e[16:24, :] * inv_e, acc_o[0:8, :] * inv_o)
        ot_scr[pl.ds(r0 + 24, 16), :] = acc_o[8:24, :] * inv_o

    def body(it, carry):
        m, mrun = carry
        h0 = it * HPI
        wrap = h0 + HPI >= H
        tn = jnp.where(wrap, jnp.minimum(step + 1, NQ - 1), step)
        hn = jnp.where(wrap, 0, h0 + HPI)
        fcols = pl.ds(pl.multiple_of(it * FL, FL), FL)

        def ffn_up():
            xn = xn_scr[pl.ds(q0, TQ), :]
            g = jnp.dot(xn, wg_ref[:, fcols], preferred_element_type=F32)
            u = jnp.dot(xn, wu_ref[:, fcols], preferred_element_type=F32)
            return (g * jax.nn.sigmoid(g) * u).astype(BF16)

        def ffn_down(hidden):
            part = jnp.dot(hidden, wd_ref[fcols, :], preferred_element_type=F32)
            prev = jnp.where(it == 0, x_ref[pl.ds(q0, TQ), :].astype(F32), y_scr[...])
            y_scr[...] = prev + part

        m_next = m
        accs = []
        parts = []
        acc = None
        cur = None
        for t in range(HPI * NCK):
            if t == 0:
                hidden = ffn_up()
            elif t == 1:
                ffn_down(hidden)
            u = t + NCS + LEAD
            i1, c1 = divmod(u, NCK)
            if cur is None or c1 == 0:
                h1, t1 = (h0 + i1, step) if i1 < HPI else (hn + (i1 - HPI), tn)
                cur = item_q(h1, pl.multiple_of(t1 * TQ, TQ))
                vinfo = (h1, q_rows(h1, i1 % 2, t1))
            if u % NCS == 0:
                mrun = None
            mrun = stage1_chunk(u // NCS, cur[0], cur[1], c1, mrun, vinfo)
            if u % NCS == NCS - 1:
                m_range = jnp.max(mrun, axis=0, keepdims=True)
                m_next = m_range if c1 < NCS else jnp.maximum(m_next, m_range)
            i2, c2 = divmod(t, NCK)
            acc = stage2_chunk(t // NCS, h0 + i2, m, c2, m_scr[16:40, :] if t % NCS == 0 else acc)
            if t % NCS == NCS - 1:
                parts.append((m, acc))
                m = m_next
            if c2 == NCK - 1:
                mt, tot = parts[-1]
                for pm, pa in parts[:-1]:
                    tot = tot + pa * jnp.exp2(pm - mt)
                parts = []
                accs.append(tot)
                if i2 % 2 == 1:
                    finish_pair((h0 + i2) // 2, accs[-2], accs[-1])
        return m, mrun

    m_fin, mrun_fin = lax.fori_loop(0, H // HPI, body, (m_scr[0:1, :], m_scr[8:16, :]))
    m_scr[0:8, :] = jnp.broadcast_to(m_fin, (8, TQ))
    m_scr[8:16, :] = mrun_fin

    @pl.when(step > 0)
    def _():
        for j in range(TQ // TO):
            o_copy(j, q0 - TQ).wait()

    f0 = FL * (H // HPI)
    xn = xn_scr[pl.ds(q0, TQ), :]
    g = jnp.dot(xn, wg_ref[:, f0:F], preferred_element_type=F32)
    u = jnp.dot(xn, wu_ref[:, f0:F], preferred_element_type=F32)
    hid = (g * jax.nn.sigmoid(g) * u).astype(BF16)
    for j in range(TQ // TO):
        o = ot_scr[:, j * TO:(j + 1) * TO].T.astype(BF16)
        attn = jnp.dot(o, wo_ref[...], preferred_element_type=F32)
        attn = attn + jnp.dot(hid[j * TO:(j + 1) * TO, :], wd_ref[f0:F, :], preferred_element_type=F32)
        o_scr[j * TO:(j + 1) * TO, :] = (y_scr[j * TO:(j + 1) * TO, :] + attn).astype(BF16)
        o_copy(j, q0).start()

    @pl.when(step == NQ - 1)
    def _():
        for j in range(TQ // TO):
            o_copy(j, q0).wait()


@jax.jit
def pallas_parallel_sum__mha_block__swiglu_ffn__prompt_kernel(
    A_x: jax.Array,
    A_wqkv: jax.Array,
    A_wo: jax.Array,
    B_x: jax.Array,
    B_w_gate: jax.Array,
    B_w_up: jax.Array,
    B_w_down: jax.Array,
):
    del B_x
    x = A_x.reshape(S, D)
    hbm = pl.BlockSpec(memory_space=pl.ANY)
    out = pl.pallas_call(
        _kernel,
        grid=(NQ,),
        in_specs=[hbm] * 6,
        out_specs=hbm,
        out_shape=jax.ShapeDtypeStruct((S, D), A_x.dtype),
        scratch_shapes=[
            pltpu.VMEM((S, D), BF16),
            pltpu.VMEM((D, 3 * D), BF16),
            pltpu.VMEM((D, D), BF16),
            pltpu.VMEM((D, F), BF16),
            pltpu.VMEM((D, F), BF16),
            pltpu.VMEM((F, D), BF16),
            pltpu.SemaphoreType.DMA((NR + 7,)),
            pltpu.VMEM((S, D), BF16),
            pltpu.VMEM((NGX, S, 128), BF16),
            pltpu.VMEM((NGX, S, 128), BF16),
            pltpu.VMEM((H * 24, S), F32),
            pltpu.VMEM((2, S // NSP, TQ), F32),
            pltpu.VMEM((D, TQ), F32),
            pltpu.VMEM((48, TQ), F32),
            pltpu.VMEM((TQ, D), F32),
            pltpu.VMEM((TQ, D), BF16),
            pltpu.SemaphoreType.DMA((TQ // TO,)),
            pltpu.VMEM((H // 2 * NQ, 2 * DH, TQ), F32),
            pltpu.VMEM((NCK, D * NV, 128), F32),
            pltpu.VMEM((NR, NV, D), U32),
        ],
        compiler_params=pltpu.CompilerParams(
            dimension_semantics=("arbitrary",),
            vmem_limit_bytes=112 * 1024 * 1024,
        ),
    )(x, A_wqkv, A_wo, B_w_gate, B_w_up, B_w_down)
    return out.reshape(1, S, D)
```
